```python
import jax
import jax.numpy as jnp

def _softmax(x, axis=-1):
    return jax.nn.softmax(x, axis=axis)
def _gelu(x):
    return jax.nn.gelu(x, approximate=True)
def _silu(x):
    return jax.nn.silu(x)
def _sigmoid(x):
    return jax.nn.sigmoid(x)
def _layernorm(x, axis=-1, eps=1e-5):
    m = jnp.mean(x, axis=axis, keepdims=True)
    v = jnp.var(x, axis=axis, keepdims=True)
    return (x - m) / jnp.sqrt(v + eps)
def _scatter_add(tgt, idx, src, axis=0):
    return tgt.at[idx].add(src)
def _segment_sum(src, seg, n):
    return jax.ops.segment_sum(src, seg, n)
class _Rng:
    def __init__(self, key):
        self._k = key
    def _next(self):
        self._k, sub = jax.random.split(self._k)
        return sub
    def normal(self, shape):
        return jax.random.normal(self._next(), shape, dtype=jnp.bfloat16)
    def randint(self, lo, hi, shape):
        return jax.random.randint(self._next(), shape, lo, hi, dtype=jnp.int32)
    def uniform(self, shape, lo=0.0, hi=1.0):
        return jax.random.uniform(self._next(), shape, jnp.bfloat16, lo, hi)
    def permutation(self, n):
        return jax.random.permutation(self._next(), n)


kernel_name = 'interleave_layers__sliding_local_dilated__dense_activation_squared_relu__prompt'

def setup_inputs():
    _rng = _Rng(jax.random.key(int.from_bytes(__import__("os").urandom(4), "little")))
    _w = (lambda a: (lambda t: t.astype(jnp.bfloat16) if jnp.issubdtype(t.dtype, jnp.floating) else t)(jnp.asarray(a)))
    def _A_setup():
        B, S, D = 1, 2048, 1024
        return {
            "x": _w((lambda *s: _rng.normal(s) * 0.05)(B, S, D)),
            "wqkv": _w((lambda *s: _rng.normal(s) * 0.05)(D, 3 * D)),
            "wo": _w((lambda *s: _rng.normal(s) * 0.05)(D, D)),
        }
    _A_in = _A_setup()

    def _B_setup():
        B, S, D, F = 1, 2048, 1024, 3584
        return {
            "x": _w((lambda *s: _rng.normal(s) * 0.05)(B, S, D)),
            "w1": _w((lambda *s: _rng.normal(s) * 0.05)(D, F)),
            "b1": _w((lambda *s: _rng.normal(s) * 0.05)(F)),
            "w2": _w((lambda *s: _rng.normal(s) * 0.05)(F, D)),
            "b2": _w((lambda *s: _rng.normal(s) * 0.05)(D)),
        }
    _B_in = _B_setup()

    return {
        "A_x": _A_in["x"],
        "A_wqkv": _A_in["wqkv"],
        "A_wo": _A_in["wo"],
        "B_x": _B_in["x"],
        "B_w1": _B_in["w1"],
        "B_b1": _B_in["b1"],
        "B_w2": _B_in["w2"],
        "B_b2": _B_in["b2"],
    }

def reference(A_x, A_wqkv, A_wo, B_x, B_w1, B_b1, B_w2, B_b2):
    def _A_ref(x, wqkv, wo):
        B, S, D = x.shape
        H = 32; Dh = D // H
        W, dil = 8, 2
        qkv = (lambda x, *d: x.transpose(*d))((x @ wqkv).reshape(B, S, 3, H, Dh), 2, 0, 3, 1, 4)
        q, k, v = qkv[0], qkv[1], qkv[2]
        scale = Dh ** -0.5
        pos = jnp.arange(S)
        off = jnp.arange(W) * dil
        idx = pos[:, None] - off[None, :]
        mask = idx >= 0
        idx_c = jnp.where(mask, idx, 0).reshape(-1)
        kg = k[:, :, idx_c, :].reshape(B, H, S, W, Dh)
        vg = v[:, :, idx_c, :].reshape(B, H, S, W, Dh)
        logits = jnp.einsum("bhsd,bhswd->bhsw", q, kg) * scale
        logits = jnp.where(mask[None, None, :, :], logits, -1e9)
        attn = _softmax(logits, axis=-1)
        o = jnp.einsum("bhsw,bhswd->bhsd", attn, vg)
        return (lambda x, *d: x.transpose(*d))(o, 0, 2, 1, 3).reshape(B, S, D) @ wo

    def _B_ref(x, w1, b1, w2, b2):
        h = jnp.einsum("bsd,df->bsf", x, w1) + b1
        zero = jnp.zeros_like(h)
        r = jnp.where(h > zero, h, zero)
        h = r * r
        out = jnp.einsum("bsf,fd->bsd", h, w2) + b2
        return out

    x = A_x
    x = x + _A_ref(_layernorm(x, axis=-1), A_wqkv, A_wo)
    x = x + _B_ref(_layernorm(x, axis=-1), B_w1, B_b1, B_w2, B_b2)
    x = x + _A_ref(_layernorm(x, axis=-1), A_wqkv, A_wo)
    x = x + _B_ref(_layernorm(x, axis=-1), B_w1, B_b1, B_w2, B_b2)
    return x
```

```python
import functools
import numpy as np
import jax
import jax.numpy as jnp
from jax import lax
import jax.experimental.pallas as pl
import jax.experimental.pallas.tpu as pltpu

S, D, F, H, DH = 2048, 1024, 3584, 32, 32
WIN, DIL = 8, 2
EPS = 1e-5
F32, BF16, U32 = jnp.float32, jnp.bfloat16, jnp.uint32

NN = (((1,), (0,)), ((), ()))
NT = (((1,), (1,)), ((), ()))


def _dot(a, b, dims=NN):
    return lax.dot_general(a, b, dims, preferred_element_type=F32)


def _ln(x):
    m = jnp.mean(x, axis=-1, keepdims=True)
    c = x - m
    v = jnp.mean(c * c, axis=-1, keepdims=True)
    return c * lax.rsqrt(v + EPS)


def _unpack(w):
    lo = pltpu.unpack_elementwise(w, index=0, packed_dtype=BF16, unpacked_dtype=F32)
    hi = pltpu.unpack_elementwise(w, index=1, packed_dtype=BF16, unpacked_dtype=F32)
    return lo, hi


def _pk(x):
    return pltpu.bitcast(x.astype(BF16), U32)


def _bf(w):
    return pltpu.bitcast(w, BF16)


def make(R=256, HG=4, LNC=64, NL=2, WOS=4, LNA=0, LNB=0):
    NB = S // R
    T = R // 128
    GR = HG * DH
    GP = GR // 2
    NG = D // GR
    ND = GR // 8
    NP = ND // 2

    def kernel(x_hbm, wqkv_hbm, wo_hbm, w1_hbm, b1_ref, w2_hbm, b2_ref, out_hbm,
               xin, wqkv_raw, wo_raw, wt, wo, w1, w2, bb1, bb2, xa, xb, xn, qkv, kprev, vprev, o, h, ostage,
               sem_x, sem_qkv, sem_w, sem_o, sem_c):
        cp_q = [[pltpu.make_async_copy(wqkv_hbm.at[:, pl.ds(p * D + g * GR, GR)],
                                       wqkv_raw.at[:, pl.ds(p * D + g * GR, GR)],
                                       sem_qkv.at[g * 3 + p]) for p in range(3)] for g in range(NG)]

        def blk(i):
            return pl.ds(i * R if isinstance(i, int) else pl.multiple_of(i * R, R), R)

        def cp_x(i):
            return pltpu.make_async_copy(x_hbm.at[blk(i)], xin.at[blk(i)], sem_x.at[i])

        def cp_o(i):
            return pltpu.make_async_copy(ostage.at[blk(i)], out_hbm.at[blk(i)], sem_o.at[i])

        cp_ba = pltpu.make_async_copy(xb.at[blk(0)], xa.at[blk(NB)], sem_c.at[0])
        cp_ab = pltpu.make_async_copy(xa.at[blk(0)], xb.at[blk(NB)], sem_c.at[1])

        cp_wo = pltpu.make_async_copy(wo_hbm, wo_raw, sem_w.at[0])
        cp_w1 = pltpu.make_async_copy(w1_hbm, w1, sem_w.at[1])
        cp_w2 = pltpu.make_async_copy(w2_hbm, w2, sem_w.at[2])
        cp_x(0).start()
        for g in range(NG):
            for p in range(3):
                cp_q[g][p].start()
        cp_wo.start()
        cp_x(1).start()

        kprev[...] = jnp.zeros_like(kprev)
        vprev[...] = jnp.zeros_like(vprev)
        bb1[...] = jnp.broadcast_to(b1_ref[...].astype(F32).reshape(1, F), (8, F))
        bb2[...] = jnp.broadcast_to(b2_ref[...].astype(F32).reshape(1, D), (8, D))

        rp = lax.broadcasted_iota(jnp.int32, (GR, GR), 0)
        cc = lax.broadcasted_iota(jnp.int32, (GR, GR), 1)
        jj = 2 * (rp // 16) + rp % 2
        ss = (rp % 16) // 2
        src = (ss % HG) * DH + (ss // HG) * ND + jj
        P = jnp.where(src == cc, 1.0, 0.0).astype(BF16)
        srco = (rp % HG) * DH + ((rp % 8) // HG) * ND + rp // 8
        Po = jnp.where(srco == cc, 1.0, 0.0).astype(BF16)

        def convert(i):
            xa[blk(i), :] = xin[blk(i), :].astype(F32)

        def layernorm(src_ref, i, lo=0, hi=R):
            for c in range(lo // LNC, hi // LNC):
                r = i * R + c * LNC
                r = r if isinstance(r, int) else pl.multiple_of(r, LNC)
                xn[pl.ds(c * LNC // 2, LNC // 2), :] = _pk(_ln(src_ref[pl.ds(r, LNC), :]))

        cp_x(0).wait()
        convert(0)
        layernorm(xa, 0)
        for g in range(NG):
            for p in range(3):
                cp_q[g][p].wait()
                wt[pl.ds((g * 3 + p) * GP, GP), :] = _pk(_dot(
                    P, wqkv_raw[:, pl.ds(p * D + g * GR, GR)], NT))
        cp_w1.start()
        cp_w2.start()
        for i in range(2, NB):
            cp_x(i).start()
        cp_wo.wait()
        for g in range(NG):
            wo[pl.ds(g * GP, GP), :] = _pk(_dot(Po, wo_raw[pl.ds(g * GR, GR), :]))

        lane = lax.broadcasted_iota(jnp.int32, (8, 128), 1)

        def attention(g, first):
            base = g * 3 * GP
            for t in range(T):
                cols = pl.ds(t * 128, 128)

                def shifted(part, prev_ref, d):
                    rows = pl.ds(base + part * GP + d * 8, 8)
                    cur = qkv[rows, cols]
                    if t == 0:
                        prev = prev_ref[pl.ds(g * GP + d * 8, 8), :]
                        if part == 2:
                            prev = jnp.where(first, jnp.broadcast_to(cur[:, 0:1], (8, 128)), prev)
                    else:
                        prev = qkv[rows, pl.ds((t - 1) * 128, 128)]
                    out = [_unpack(cur)]
                    for w in range(1, WIN):
                        sh = w * DIL
                        out.append(_unpack(pltpu.roll(jnp.where(lane >= 128 - sh, prev, cur), sh, 1)))
                    return out

                acc = [None] * WIN
                for d in range(NP):
                    q0, q1 = _unpack(qkv[pl.ds(base + d * 8, 8), cols])
                    ks = shifted(1, kprev, d)
                    for w in range(WIN):
                        pr = q0 * ks[w][0] + q1 * ks[w][1]
                        acc[w] = pr if acc[w] is None else acc[w] + pr
                r = HG
                while r < 8:
                    acc = [a + pltpu.roll(a, r, 0) for a in acc]
                    r *= 2
                lg = [a * (DH ** -0.5) for a in acc]
                if t == 0:
                    lg = [lg[0]] + [jnp.where(jnp.logical_and(first, lane < w * DIL), -1e9, lg[w])
                                    for w in range(1, WIN)]
                m = functools.reduce(jnp.maximum, lg)
                e = [jnp.exp(a - m) for a in lg]
                inv = 1.0 / functools.reduce(jnp.add, e)
                p = [a * inv for a in e]
                outs = []
                for d in range(NP):
                    vs = shifted(2, vprev, d)
                    os_ = []
                    for k in range(2):
                        acc_o = p[0] * vs[0][k]
                        for w in range(1, WIN):
                            acc_o = acc_o + p[w] * vs[w][k]
                        os_.append(acc_o)
                    outs.append(jnp.concatenate(os_, axis=0).astype(BF16))
                oT = jnp.concatenate(outs, axis=0)
                o[pl.ds(t * 64, 64), pl.ds(g * GR, GR)] = pltpu.bitcast(oT.T, U32)
            last = pl.ds((T - 1) * 128, 128)
            kprev[pl.ds(g * GP, GP), :] = qkv[pl.ds(base + GP, GP), last]
            vprev[pl.ds(g * GP, GP), :] = qkv[pl.ds(base + 2 * GP, GP), last]

        def attn_unit(i, l):
            @pl.when(jnp.logical_and(l == 0, i + 1 < NB))
            def _():
                cp_x(i + 1).wait()
                convert(i + 1)

            @pl.when(i == 1)
            def _():
                cp_ba.start()

            @pl.when(i == NB - 1)
            def _():
                cp_ba.wait()

            first = i == 0

            def proj(g):
                y = _dot(_bf(wt[pl.ds(g * 3 * GP, 3 * GP), :]), _bf(xn[...]), NT)
                qkv[pl.ds(g * 3 * GP, 3 * GP), :] = _pk(y)

            proj(0)
            for g in range(NG - 1):
                proj(g + 1)
                attention(g, first)
            if WOS:
                k1 = WOS * GR
                y = _dot(_bf(o[:, :k1]), _bf(wo[:k1 // 2, :]))
                xb[blk(i), :] = xa[blk(i), :] + y
                attention(NG - 1, first)
                layernorm(xa, i + 1)
                y = _dot(_bf(o[:, k1:]), _bf(wo[k1 // 2:, :]))
                xb[blk(i), :] = xb[blk(i), :] + y
            else:
                attention(NG - 1, first)
                layernorm(xa, i + 1)
                y = _dot(_bf(o[...]), _bf(wo[...]))
                xb[blk(i), :] = xa[blk(i), :] + y

        def ffn_unit(i, l):
            @pl.when(i == 1)
            def _():
                cp_ab.start()

            @pl.when(i == NB - 1)
            def _():
                cp_ab.wait()

            hh = _dot(_bf(xn[...]), w1[...]) + bb1[0:1, :]
            rr = jnp.where(hh > 0, hh, 0.0)
            h[...] = _pk(rr * rr)
            if LNB == 0:
                layernorm(xb, i + 1)
                x2 = xb[blk(i), :] + (_dot(_bf(h[...]), w2[...]) + bb2[0:1, :])
                xa[blk(i), :] = x2
                ostage[blk(i), :] = x2.astype(BF16)
            else:
                NC = D // LNB
                for c in range(LNB):
                    cs = pl.ds(c * NC, NC)
                    layernorm(xb, i + 1, c * R // LNB, (c + 1) * R // LNB)
                    x2 = xb[blk(i), cs] + (_dot(_bf(h[...]), w2[:, cs]) + bb2[0:1, cs])
                    xa[blk(i), cs] = x2
                    ostage[blk(i), cs] = x2.astype(BF16)

            @pl.when(l == NL - 1)
            def _():
                cp_o(i).start()

        def layer(l, carry):
            def _a(i, c):
                with jax.named_scope("attn_unit"):
                    attn_unit(i, l)
                return c
            lax.fori_loop(0, NB, _a, 0)

            @pl.when(l == 0)
            def _():
                with jax.named_scope("wait_w"):
                    cp_w1.wait()
                    cp_w2.wait()

            def _b(i, c):
                with jax.named_scope("ffn_unit"):
                    ffn_unit(i, l)
                return c
            lax.fori_loop(0, NB, _b, 0)
            return carry

        lax.fori_loop(0, NL, layer, 0)
        with jax.named_scope("wait_o"):
            for i in range(NB):
                cp_o(i).wait()

    def run(A_x, A_wqkv, A_wo, B_x, B_w1, B_b1, B_w2, B_b2):
        del B_x
        hbm = pl.BlockSpec(memory_space=pl.ANY)
        vm = pl.BlockSpec(memory_space=pltpu.VMEM)
        out = pl.pallas_call(
            kernel,
            out_shape=jax.ShapeDtypeStruct((S, D), BF16),
            in_specs=[hbm, hbm, hbm, hbm, vm, hbm, vm],
            out_specs=hbm,
            scratch_shapes=[
                pltpu.VMEM((S, D), BF16),
                pltpu.VMEM((D, 3 * D), BF16),
                pltpu.VMEM((D, D), BF16),
                pltpu.VMEM((3 * D // 2, D), U32),
                pltpu.VMEM((D // 2, D), U32),
                pltpu.VMEM((D, F), BF16),
                pltpu.VMEM((F, D), BF16),
                pltpu.VMEM((8, F), F32),
                pltpu.VMEM((8, D), F32),
                pltpu.VMEM((S + R, D), F32),
                pltpu.VMEM((S + R, D), F32),
                pltpu.VMEM((R // 2, D), U32),
                pltpu.VMEM((3 * D // 2, R), U32),
                pltpu.VMEM((D // 2, 128), U32),
                pltpu.VMEM((D // 2, 128), U32),
                pltpu.VMEM((R // 2, D), U32),
                pltpu.VMEM((R // 2, F), U32),
                pltpu.VMEM((S, D), BF16),
                pltpu.SemaphoreType.DMA((NB,)),
                pltpu.SemaphoreType.DMA((3 * NG,)),
                pltpu.SemaphoreType.DMA((3,)),
                pltpu.SemaphoreType.DMA((NB,)),
                pltpu.SemaphoreType.DMA((2,)),
            ],
            compiler_params=pltpu.CompilerParams(vmem_limit_bytes=110 * 1024 * 1024),
        )(A_x.reshape(S, D), A_wqkv, A_wo, B_w1, B_b1, B_w2, B_b2)
        return out.reshape(1, S, D)

    return run


@jax.jit
def pallas_interleave_layers__sliding_local_dilated__dense_activation_squared_relu__prompt_kernel(A_x, A_wqkv, A_wo, B_x, B_w1, B_b1, B_w2, B_b2):
    return make(WOS=4,LNB=0)(A_x, A_wqkv, A_wo, B_x, B_w1, B_b1, B_w2, B_b2)
```

```python
import functools
import numpy as np
import jax
import jax.numpy as jnp
from jax import lax
import jax.experimental.pallas as pl
import jax.experimental.pallas.tpu as pltpu

S, D, F, H, DH = 2048, 1024, 3584, 32, 32
WIN, DIL = 8, 2
EPS = 1e-5
F32, BF16, U32 = jnp.float32, jnp.bfloat16, jnp.uint32

NN = (((1,), (0,)), ((), ()))
NT = (((1,), (1,)), ((), ()))


def _dot(a, b, dims=NN):
    return lax.dot_general(a, b, dims, preferred_element_type=F32)


def _ln(x):
    m = jnp.mean(x, axis=-1, keepdims=True)
    c = x - m
    v = jnp.mean(c * c, axis=-1, keepdims=True)
    return c * lax.rsqrt(v + EPS)


def _unpack(w):
    lo = pltpu.unpack_elementwise(w, index=0, packed_dtype=BF16, unpacked_dtype=F32)
    hi = pltpu.unpack_elementwise(w, index=1, packed_dtype=BF16, unpacked_dtype=F32)
    return lo, hi


def _pk(x):
    return pltpu.bitcast(x.astype(BF16), U32)


def _bf(w):
    return pltpu.bitcast(w, BF16)


def make(R=256, LNC=64, NL=2, WOS=4, WT=0, WAITS=(0, 1, 2, 3, 4, 5, 6, 7), AHEAD=2, AF=(0, 1), XNB=1, LNE=1):
    NB = S // R
    T = R // 128
    GR = 128
    GP = GR // 2
    NG = D // GR
    NP = GP // 8

    def kernel(x_hbm, wqkv_hbm, wo_hbm, w1_hbm, b1_ref, w2_hbm, b2_ref, out_hbm,
               xin, wqkv, wt, wo, w1, w2, bb1, bb2, xa, xb, xn, qkv, kprev, vprev, o, h, ostage,
               sem_x, sem_qkv, sem_w, sem_o, sem_c):
        cp_q = [[pltpu.make_async_copy(wqkv_hbm.at[:, pl.ds(p * D + g * GR, GR)],
                                       wqkv.at[:, pl.ds(p * D + g * GR, GR)],
                                       sem_qkv.at[g * 3 + p]) for p in range(3)] for g in range(NG)]

        def blk(i):
            return pl.ds(i * R if isinstance(i, int) else pl.multiple_of(i * R, R), R)

        def cp_x(i):
            return pltpu.make_async_copy(x_hbm.at[blk(i)], xin.at[blk(i)], sem_x.at[i])

        def cp_o(i):
            return pltpu.make_async_copy(ostage.at[blk(i)], out_hbm.at[blk(i)], sem_o.at[i])

        cp_ba = pltpu.make_async_copy(xb.at[blk(0)], xa.at[blk(NB)], sem_c.at[0])
        cp_ab = pltpu.make_async_copy(xa.at[blk(0)], xb.at[blk(NB)], sem_c.at[1])

        cp_wo = pltpu.make_async_copy(wo_hbm, wo, sem_w.at[0])
        cp_w1 = pltpu.make_async_copy(w1_hbm, w1, sem_w.at[1])
        cp_w2 = pltpu.make_async_copy(w2_hbm, w2, sem_w.at[2])

        queue = [[cp_x(0)]] + cp_q + [[cp_x(1), cp_wo]]
        issued = [0]

        def issue(n):
            while issued[0] < min(n, len(queue)):
                for c in queue[issued[0]]:
                    c.start()
                issued[0] += 1

        issue(2)

        kprev[...] = jnp.zeros_like(kprev)
        vprev[...] = jnp.zeros_like(vprev)
        bb1[...] = jnp.broadcast_to(b1_ref[...].astype(F32).reshape(1, F), (8, F))
        bb2[...] = jnp.broadcast_to(b2_ref[...].astype(F32).reshape(1, D), (8, D))

        XN0 = S + R

        def get_xn():
            return pltpu.bitcast(xb[pl.ds(XN0, R // 2), :], BF16) if XNB else _bf(xn[...])

        def convert(i):
            xa[blk(i), :] = xin[blk(i), :].astype(F32)

        def layernorm(src_ref, i, lo=0, hi=R):
            for c in range(lo // LNC, hi // LNC):
                r = i * R + c * LNC
                r = r if isinstance(r, int) else pl.multiple_of(r, LNC)
                y = _ln(src_ref[pl.ds(r, LNC), :])
                if XNB:
                    xb[pl.ds(XN0 + c * LNC // 2, LNC // 2), :] = pltpu.bitcast(y.astype(BF16), F32)
                else:
                    xn[pl.ds(c * LNC // 2, LNC // 2), :] = _pk(y)

        QX0 = 3 * D // 2
        NQ = D // R

        def layernorm_staged(i, zero):
            for c in range(R // LNC):
                r = pl.multiple_of(i * R + c * LNC, LNC)
                y = _pk(_ln(xa[pl.ds(r, LNC), :]))
                for k in range(NQ):
                    r2 = pl.multiple_of(zero + QX0 + k * (R // 2) + c * LNC // 2, 8)
                    qkv[pl.ds(r2, LNC // 2), :] = y[:, k * R:(k + 1) * R]

        def unstage():
            for k in range(NQ):
                xb[pl.ds(XN0, R // 2), pl.ds(k * R, R)] = pltpu.bitcast(
                    qkv[pl.ds(QX0 + k * (R // 2), R // 2), :], F32)

        lane = lax.broadcasted_iota(jnp.int32, (8, 128), 1)
        sub = lax.broadcasted_iota(jnp.int32, (8, 128), 0)
        m_even = (sub & 2) == 0
        m_odd = ((sub + 7) & 2) == 0
        m_par = (sub & 1) == 0

        def fold(a):
            u = jnp.where(m_even, a[0], a[2]) + pltpu.roll(jnp.where(m_even, a[2], a[0]), 6, 0)
            v = jnp.where(m_odd, a[1], a[3]) + pltpu.roll(jnp.where(m_odd, a[3], a[1]), 6, 0)
            z = jnp.where(m_par, u, v) + pltpu.roll(jnp.where(m_par, v, u), 7, 0)
            return z + pltpu.roll(z, 4, 0)

        def attention(g, first):
            base = g * 3 * GP
            for t in range(T):
                cols = pl.ds(t * 128, 128)

                def shifted(part, prev_ref, d):
                    rows = pl.ds(base + part * GP + d * 8, 8)
                    cur = qkv[rows, cols]
                    if t == 0:
                        if first is True:
                            prev = jnp.broadcast_to(cur[:, 0:1], (8, 128))
                        else:
                            prev = prev_ref[pl.ds(g * GP + d * 8, 8), :]
                            if part == 2:
                                prev = jnp.where(first, jnp.broadcast_to(cur[:, 0:1], (8, 128)), prev)
                    else:
                        prev = qkv[rows, pl.ds((t - 1) * 128, 128)]
                    out = [_unpack(cur)]
                    for w in range(1, WIN):
                        sh = w * DIL
                        out.append(_unpack(pltpu.roll(jnp.where(lane >= 128 - sh, prev, cur), sh, 1)))
                    return out

                acc = [[None] * 4 for _ in range(WIN)]
                for d in range(NP):
                    hd = d // 2
                    q0, q1 = _unpack(qkv[pl.ds(base + d * 8, 8), cols])
                    ks = shifted(1, kprev, d)
                    for w in range(WIN):
                        pr = q0 * ks[w][0] + q1 * ks[w][1]
                        acc[w][hd] = pr if acc[w][hd] is None else acc[w][hd] + pr
                lg = [fold(a) * (DH ** -0.5) for a in acc]
                if t == 0:
                    lg = [lg[0]] + [jnp.where(jnp.logical_and(first, lane < w * DIL), -1e9, lg[w])
                                    for w in range(1, WIN)]
                m = functools.reduce(jnp.maximum, lg)
                e = [jnp.exp(a - m) for a in lg]
                inv = 1.0 / functools.reduce(jnp.add, e)
                p = [a * inv for a in e]
                outs = []
                for d in range(NP):
                    hd = d // 2
                    if d % 2 == 0:
                        ph = [jnp.broadcast_to(a[hd:hd + 1, :], (8, 128)) for a in p]
                    vs = shifted(2, vprev, d)
                    os_ = []
                    for k in range(2):
                        acc_o = ph[0] * vs[0][k]
                        for w in range(1, WIN):
                            acc_o = acc_o + ph[w] * vs[w][k]
                        os_.append(acc_o)
                    outs.append(_bf(pltpu.pack_elementwise(os_, packed_dtype=BF16)))
                oT = jnp.concatenate(outs, axis=0)
                o[pl.ds(t * 64, 64), pl.ds(g * GR, GR)] = pltpu.bitcast(oT.T, U32)
            last = pl.ds((T - 1) * 128, 128)
            kprev[pl.ds(g * GP, GP), :] = qkv[pl.ds(base + GP, GP), last]
            vprev[pl.ds(g * GP, GP), :] = qkv[pl.ds(base + 2 * GP, GP), last]

        def attn_unit(i, peeled=False):
            first = True if peeled else i == 0

            def transpose_w(g):
                for p in range(3):
                    wt[pl.ds((g * 3 + p) * GP, GP), :] = pltpu.bitcast(wqkv[:, pl.ds(p * D + g * GR, GR)].T, U32)

            waited = [0]

            def need(g):
                if peeled and waited[0] <= min(g, NG - 1):
                    nxt = min([w for w in WAITS if w > g] + [NG])
                    for gg in range(waited[0], nxt):
                        for c in cp_q[gg]:
                            c.wait()
                        issue(gg + 2 + AHEAD)
                        if WT:
                            transpose_w(gg)
                    waited[0] = nxt

            def proj(g):
                need(g)
                if WT:
                    y = _dot(_bf(wt[pl.ds(g * 3 * GP, 3 * GP), :]), get_xn(), NT)
                    qkv[pl.ds(g * 3 * GP, 3 * GP), :] = _pk(y)
                else:
                    for p in range(3):
                        y = _dot(get_xn(), wqkv[:, pl.ds(p * D + g * GR, GR)]).astype(BF16)
                        qkv[pl.ds((g * 3 + p) * GP, GP), :] = pltpu.bitcast(y.T, U32)

            early = LNE and not peeled
            if early:
                layernorm_staged(i + 1, i >> 8)
            proj(0)
            for g in range(NG - 1):
                if AF[int(peeled)]:
                    need(g + 1)
                    attention(g, first)
                    proj(g + 1)
                else:
                    proj(g + 1)
                    attention(g, first)
            if peeled:
                cp_x(1).wait()
                cp_wo.wait()
                cp_w1.start()
                cp_w2.start()
                for j in range(2, NB):
                    cp_x(j).start()
                convert(1)
            k1 = WOS * GR
            y = _dot(_bf(o[:, :k1]), wo[:k1, :])
            xb[blk(i), :] = xa[blk(i), :] + y
            attention(NG - 1, first)
            if early:
                unstage()
            else:
                layernorm(xa, i + 1)
            y = _dot(_bf(o[:, k1:]), wo[k1:, :])
            xb[blk(i), :] = xb[blk(i), :] + y

        def ffn_unit(i, l):
            @pl.when(i == 1)
            def _():
                cp_ab.start()

            @pl.when(i == NB - 1)
            def _():
                cp_ab.wait()

            hh = _dot(get_xn(), w1[...]) + bb1[0:1, :]
            rr = jnp.where(hh > 0, hh, 0.0)
            h[...] = _pk(rr * rr)
            layernorm(xb, i + 1)
            x2 = xb[blk(i), :] + (_dot(_bf(h[...]), w2[...]) + bb2[0:1, :])
            xa[blk(i), :] = x2
            ostage[blk(i), :] = x2.astype(BF16)

            @pl.when(l == NL - 1)
            def _():
                cp_o(i).start()

        cp_x(0).wait()
        issue(1 + AHEAD)
        convert(0)
        layernorm(xa, 0)
        with jax.named_scope("attn_first"):
            attn_unit(0, True)

        def layer(l, carry):
            def _a(i, c):
                @pl.when(jnp.logical_and(l == 0, i + 1 < NB))
                def _():
                    cp_x(i + 1).wait()
                    convert(i + 1)

                @pl.when(i == 1)
                def _():
                    cp_ba.start()

                @pl.when(i == NB - 1)
                def _():
                    cp_ba.wait()

                with jax.named_scope("attn_unit"):
                    attn_unit(i)
                return c
            lax.fori_loop(jnp.where(l == 0, 1, 0), NB, _a, 0)

            @pl.when(l == 0)
            def _():
                with jax.named_scope("wait_w"):
                    cp_w1.wait()
                    cp_w2.wait()

            def _b(i, c):
                with jax.named_scope("ffn_unit"):
                    ffn_unit(i, l)
                return c
            lax.fori_loop(0, NB, _b, 0)
            return carry

        lax.fori_loop(0, NL, layer, 0)
        with jax.named_scope("wait_o"):
            for i in range(NB):
                cp_o(i).wait()

    def run(A_x, A_wqkv, A_wo, B_x, B_w1, B_b1, B_w2, B_b2):
        del B_x
        hbm = pl.BlockSpec(memory_space=pl.ANY)
        vm = pl.BlockSpec(memory_space=pltpu.VMEM)
        out = pl.pallas_call(
            kernel,
            out_shape=jax.ShapeDtypeStruct((S, D), BF16),
            in_specs=[hbm, hbm, hbm, hbm, vm, hbm, vm],
            out_specs=hbm,
            scratch_shapes=[
                pltpu.VMEM((S, D), BF16),
                pltpu.VMEM((D, 3 * D), BF16),
                pltpu.VMEM((3 * D // 2, D) if WT else (8, 128), U32),
                pltpu.VMEM((D, D), BF16),
                pltpu.VMEM((D, F), BF16),
                pltpu.VMEM((F, D), BF16),
                pltpu.VMEM((8, F), F32),
                pltpu.VMEM((8, D), F32),
                pltpu.VMEM((S + R, D), F32),
                pltpu.VMEM((S + R + R // 2, D), F32),
                pltpu.VMEM((R // 2, D), U32),
                pltpu.VMEM((3 * D // 2 + D // 2, R), U32),
                pltpu.VMEM((D // 2, 128), U32),
                pltpu.VMEM((D // 2, 128), U32),
                pltpu.VMEM((R // 2, D), U32),
                pltpu.VMEM((R // 2, F), U32),
                pltpu.VMEM((S, D), BF16),
                pltpu.SemaphoreType.DMA((NB,)),
                pltpu.SemaphoreType.DMA((3 * NG,)),
                pltpu.SemaphoreType.DMA((3,)),
                pltpu.SemaphoreType.DMA((NB,)),
                pltpu.SemaphoreType.DMA((2,)),
            ],
            compiler_params=pltpu.CompilerParams(vmem_limit_bytes=110 * 1024 * 1024),
        )(A_x.reshape(S, D), A_wqkv, A_wo, B_w1, B_b1, B_w2, B_b2)
        return out.reshape(1, S, D)

    return run


@jax.jit
def pallas_interleave_layers__sliding_local_dilated__dense_activation_squared_relu__prompt_kernel(A_x, A_wqkv, A_wo, B_x, B_w1, B_b1, B_w2, B_b2):
    return make(WT=0,AF=(0,1),LNC=16,WAITS=(0,1,2,3,5),AHEAD=3)(A_x, A_wqkv, A_wo, B_x, B_w1, B_b1, B_w2, B_b2)
```

```python
import functools
import numpy as np
import jax
import jax.numpy as jnp
from jax import lax
import jax.experimental.pallas as pl
import jax.experimental.pallas.tpu as pltpu

S, D, F, H, DH = 2048, 1024, 3584, 32, 32
WIN, DIL = 8, 2
EPS = 1e-5
F32, BF16, U32 = jnp.float32, jnp.bfloat16, jnp.uint32

NN = (((1,), (0,)), ((), ()))


def _dot(a, b, dims=NN):
    return lax.dot_general(a, b, dims, preferred_element_type=F32)


def _ln(x):
    m = jnp.mean(x, axis=-1, keepdims=True)
    c = x - m
    v = jnp.mean(c * c, axis=-1, keepdims=True)
    return c * lax.rsqrt(v + EPS)


def _unpack(w):
    lo = pltpu.unpack_elementwise(w, index=0, packed_dtype=BF16, unpacked_dtype=F32)
    hi = pltpu.unpack_elementwise(w, index=1, packed_dtype=BF16, unpacked_dtype=F32)
    return lo, hi


def _pk(x):
    return pltpu.bitcast(x.astype(BF16), U32)


def _bf(w):
    return pltpu.bitcast(w, BF16)


def make(R=256, LNC=16, LNB=32, NL=2, WOS=4, WAITS=(0, 1, 2, 3, 4, 5, 6, 7), AHEAD=9, AF=(0, 1), DEFER=1, ORD=(0, 1, 2),
         SCOPES=False, LNP=1):
    NB = S // R
    T = R // 128
    GR = 128
    GP = GR // 2
    NG = D // GR
    NP = GP // 8
    XN0 = S + R
    QX0 = 3 * D // 2
    NQ = D // R

    def scoped(name, fn):
        if SCOPES:
            with jax.named_scope(name):
                fn()
        else:
            fn()

    def kernel(x_hbm, wqkv_hbm, wo_hbm, w1_hbm, b1_ref, w2_hbm, b2_ref, out_hbm,
               xin, wqkv, wo, w1, w2, bb1, bb2, xa, xb, qkv, kprev, vprev, o, h, tmp, ostage,
               sem_x, sem_qkv, sem_w, sem_o, sem_c):
        cp_q = [[pltpu.make_async_copy(wqkv_hbm.at[:, pl.ds(p * D + g * GR, GR)],
                                       wqkv.at[:, pl.ds(p * D + g * GR, GR)],
                                       sem_qkv.at[g * 3 + p]) for p in range(3)] for g in range(NG)]

        def rows(r, n):
            return pl.ds(r if isinstance(r, int) else pl.multiple_of(r, n), n)

        def blk(i):
            return rows(i * R, R)

        def cp_x(i):
            return pltpu.make_async_copy(x_hbm.at[blk(i)], xin.at[blk(i)], sem_x.at[i])

        def cp_o(i):
            return pltpu.make_async_copy(ostage.at[blk(i)], out_hbm.at[blk(i)], sem_o.at[i])

        cp_ba = pltpu.make_async_copy(xb.at[blk(0)], xa.at[blk(NB)], sem_c.at[0])
        cp_ab = pltpu.make_async_copy(xa.at[blk(0)], xb.at[blk(NB)], sem_c.at[1])

        k1 = WOS * GR
        cp_wo1 = pltpu.make_async_copy(wo_hbm.at[:k1], wo.at[:k1], sem_w.at[0])
        cp_wo2 = pltpu.make_async_copy(wo_hbm.at[k1:], wo.at[k1:], sem_w.at[3])
        cp_w1 = pltpu.make_async_copy(w1_hbm, w1, sem_w.at[1])
        cp_w2 = pltpu.make_async_copy(w2_hbm, w2, sem_w.at[2])

        queue = [[cp_x(0)]] + cp_q + [[cp_wo1], [cp_x(1), cp_wo2]]
        issued = [0]

        def issue(n):
            while issued[0] < min(n, len(queue)):
                for c in queue[issued[0]]:
                    c.start()
                issued[0] += 1

        issue(2)

        kprev[...] = jnp.zeros_like(kprev)
        vprev[...] = jnp.zeros_like(vprev)
        bb1[...] = jnp.broadcast_to(b1_ref[...].astype(F32).reshape(1, F), (8, F))
        bb2[...] = jnp.broadcast_to(b2_ref[...].astype(F32).reshape(1, D), (8, D))

        def get_xn():
            return pltpu.bitcast(xb[pl.ds(XN0, R // 2), :], BF16)

        def load_x(src_ref, i, off, n, from_input):
            sl = rows(i * R + off, n)
            if from_input is False:
                return src_ref[sl, :]
            if from_input is True:
                return xin[sl, :].astype(F32)
            si = rows(jnp.minimum(i, NB - 1) * R + off, n)
            return jnp.where(from_input, xin[si, :].astype(F32), src_ref[sl, :])

        def layernorm(src_ref, i, from_input=False, zero=0):
            for c in range(R // LNB):
                y = _ln(load_x(src_ref, i, c * LNB, LNB, from_input))
                xb[rows(zero + XN0 + c * LNB // 2, LNB // 2), :] = pltpu.bitcast(y.astype(BF16), F32)

        def layernorm_staged(i, zero, from_input):
            for c in range(R // LNC):
                y = _pk(_ln(load_x(xa, i, c * LNC, LNC, from_input)))
                for k in range(NQ):
                    qkv[rows(zero + QX0 + k * (R // 2) + c * LNC // 2, LNC // 2), :] = y[:, k * R:(k + 1) * R]

        def unstage():
            for k in range(NQ):
                xb[pl.ds(XN0, R // 2), pl.ds(k * R, R)] = pltpu.bitcast(
                    qkv[pl.ds(QX0 + k * (R // 2), R // 2), :], F32)

        lane = lax.broadcasted_iota(jnp.int32, (8, 128), 1)
        sub = lax.broadcasted_iota(jnp.int32, (8, 128), 0)
        m_even = (sub & 2) == 0
        m_odd = ((sub + 7) & 2) == 0
        m_par = (sub & 1) == 0

        def fold(a):
            u = jnp.where(m_even, a[0], a[2]) + pltpu.roll(jnp.where(m_even, a[2], a[0]), 6, 0)
            v = jnp.where(m_odd, a[1], a[3]) + pltpu.roll(jnp.where(m_odd, a[3], a[1]), 6, 0)
            z = jnp.where(m_par, u, v) + pltpu.roll(jnp.where(m_par, v, u), 7, 0)
            return z + pltpu.roll(z, 4, 0)

        def attention(g, first):
            base = g * 3 * GP
            for t in range(T):
                cols = pl.ds(t * 128, 128)

                def shifted(part, prev_ref, d):
                    rs = pl.ds(base + part * GP + d * 8, 8)
                    cur = qkv[rs, cols]
                    if t == 0:
                        if first is True:
                            prev = jnp.broadcast_to(cur[:, 0:1], (8, 128))
                        else:
                            prev = prev_ref[pl.ds(g * GP + d * 8, 8), :]
                            if part == 2:
                                prev = jnp.where(first, jnp.broadcast_to(cur[:, 0:1], (8, 128)), prev)
                    else:
                        prev = qkv[rs, pl.ds((t - 1) * 128, 128)]
                    out = [_unpack(cur)]
                    for w in range(1, WIN):
                        sh = w * DIL
                        out.append(_unpack(pltpu.roll(jnp.where(lane >= 128 - sh, prev, cur), sh, 1)))
                    return out

                acc = [[None] * 4 for _ in range(WIN)]
                for d in range(NP):
                    hd = d // 2
                    q0, q1 = _unpack(qkv[pl.ds(base + d * 8, 8), cols])
                    ks = shifted(1, kprev, d)
                    for w in range(WIN):
                        pr = q0 * ks[w][0] + q1 * ks[w][1]
                        acc[w][hd] = pr if acc[w][hd] is None else acc[w][hd] + pr
                lg = [fold(a) * (DH ** -0.5) for a in acc]
                if t == 0:
                    lg = [lg[0]] + [jnp.where(jnp.logical_and(first, lane < w * DIL), -1e9, lg[w])
                                    for w in range(1, WIN)]
                m = functools.reduce(jnp.maximum, lg)
                e = [jnp.exp(a - m) for a in lg]
                inv = 1.0 / functools.reduce(jnp.add, e)
                p = [a * inv for a in e]
                outs = []
                for d in range(NP):
                    hd = d // 2
                    if d % 2 == 0:
                        ph = [jnp.broadcast_to(a[hd:hd + 1, :], (8, 128)) for a in p]
                    vs = shifted(2, vprev, d)
                    os_ = []
                    for k in range(2):
                        acc_o = ph[0] * vs[0][k]
                        for w in range(1, WIN):
                            acc_o = acc_o + ph[w] * vs[w][k]
                        os_.append(acc_o)
                    outs.append(_bf(pltpu.pack_elementwise(os_, packed_dtype=BF16)))
                oT = jnp.concatenate(outs, axis=0)
                o[pl.ds(t * 64, 64), pl.ds(g * GR, GR)] = pltpu.bitcast(oT.T, U32)
            last = pl.ds((T - 1) * 128, 128)
            kprev[pl.ds(g * GP, GP), :] = qkv[pl.ds(base + GP, GP), last]
            vprev[pl.ds(g * GP, GP), :] = qkv[pl.ds(base + 2 * GP, GP), last]

        def attn_unit(i, l, peeled=False):
            first = True if peeled else i == 0
            waited = [0]
            pending = []

            def flush():
                while pending:
                    g, p = pending.pop()
                    qkv[pl.ds((g * 3 + p) * GP, GP), :] = pltpu.bitcast(_bf(tmp[...]).T, U32)

            def need(g):
                if peeled and waited[0] <= g < NG:
                    nxt = min([w for w in WAITS if w > g] + [NG])
                    issue(nxt + 1)
                    for gg in range(waited[0], nxt):
                        scoped(f"wq{gg}", lambda: [c.wait() for c in cp_q[gg]] and None)
                    issue(nxt + 1 + AHEAD)
                    waited[0] = nxt
                    flush()

            def proj(g):
                need(g)
                for p in ORD:
                    if g == 0 and p == LNP and not peeled:
                        layernorm_staged(i + 1, i >> 8, jnp.logical_and(l == 0, i + 1 < NB))
                    y = _dot(get_xn(), wqkv[:, pl.ds(p * D + g * GR, GR)]).astype(BF16)
                    if peeled and DEFER and p == ORD[-1] and (g + 1 in WAITS or g + 1 == NG):
                        tmp[...] = pltpu.bitcast(y, U32)
                        pending.append((g, p))
                    else:
                        qkv[pl.ds((g * 3 + p) * GP, GP), :] = pltpu.bitcast(y.T, U32)

            proj(0)
            for g in range(NG - 1):
                if AF[int(peeled)]:
                    need(g + 1)
                    attention(g, first)
                    proj(g + 1)
                else:
                    proj(g + 1)
                    attention(g, first)
            if peeled:
                issue(len(queue))
                scoped("wwo1", cp_wo1.wait)
                for j in range(2, NB):
                    cp_x(j).start()
                flush()
            y = _dot(_bf(o[:, :k1]), wo[:k1, :])
            xb[blk(i), :] = load_x(xa, i, 0, R, True if peeled else l == 0) + y
            attention(NG - 1, first)
            if peeled:
                scoped("wx1", cp_x(1).wait)
                scoped("wwo2", cp_wo2.wait)
                cp_w1.start()
                cp_w2.start()
                layernorm(xa, 1, True, pl.program_id(0))
            else:
                unstage()
            y = _dot(_bf(o[:, k1:]), wo[k1:, :])
            xb[blk(i), :] = xb[blk(i), :] + y

        def ffn_unit(i):
            hh = _dot(get_xn(), w1[...]) + bb1[0:1, :]
            rr = jnp.where(hh > 0, hh, 0.0)
            h[...] = _pk(rr * rr)
            layernorm(xb, i + 1)
            x2 = xb[blk(i), :] + (_dot(_bf(h[...]), w2[...]) + bb2[0:1, :])
            xa[blk(i), :] = x2
            ostage[blk(i), :] = x2.astype(BF16)

        scoped("wait_x0", lambda: cp_x(0).wait())
        issue(1 + AHEAD)
        layernorm(xa, 0, True)
        scoped("attn_first", lambda: attn_unit(0, 0, True))

        def layer(l, carry):
            def _a(i, c):
                @pl.when(jnp.logical_and(l == 0, i + 1 < NB))
                def _():
                    cp_x(i + 1).wait()

                @pl.when(i == 1)
                def _():
                    cp_ba.start()

                @pl.when(i == NB - 1)
                def _():
                    cp_ba.wait()

                scoped("attn_unit", lambda: attn_unit(i, l))
                return c
            lax.fori_loop(jnp.where(l == 0, 1, 0), NB, _a, 0)

            @pl.when(l == 0)
            def _():
                cp_w1.wait()
                cp_w2.wait()

            def _b(i, c):
                @pl.when(i == 1)
                def _():
                    cp_ab.start()

                @pl.when(i == NB - 1)
                def _():
                    cp_ab.wait()

                scoped("ffn_unit", lambda: ffn_unit(i))

                @pl.when(l == NL - 1)
                def _():
                    cp_o(i).start()
                return c
            lax.fori_loop(0, NB, _b, 0)
            return carry

        lax.fori_loop(0, NL, layer, 0)
        for i in range(NB):
            cp_o(i).wait()

    def run(A_x, A_wqkv, A_wo, B_x, B_w1, B_b1, B_w2, B_b2):
        del B_x
        hbm = pl.BlockSpec(memory_space=pl.ANY)
        vm = pl.BlockSpec(memory_space=pltpu.VMEM)
        out = pl.pallas_call(
            kernel,
            out_shape=jax.ShapeDtypeStruct((S, D), BF16),
            grid=(1,),
            in_specs=[hbm, hbm, hbm, hbm, vm, hbm, vm],
            out_specs=hbm,
            scratch_shapes=[
                pltpu.VMEM((S, D), BF16),
                pltpu.VMEM((D, 3 * D), BF16),
                pltpu.VMEM((D, D), BF16),
                pltpu.VMEM((D, F), BF16),
                pltpu.VMEM((F, D), BF16),
                pltpu.VMEM((8, F), F32),
                pltpu.VMEM((8, D), F32),
                pltpu.VMEM((S + R, D), F32),
                pltpu.VMEM((S + R + R // 2, D), F32),
                pltpu.VMEM((3 * D // 2 + D // 2, R), U32),
                pltpu.VMEM((D // 2, 128), U32),
                pltpu.VMEM((D // 2, 128), U32),
                pltpu.VMEM((R // 2, D), U32),
                pltpu.VMEM((R // 2, F), U32),
                pltpu.VMEM((R // 2, GR), U32),
                pltpu.VMEM((S, D), BF16),
                pltpu.SemaphoreType.DMA((NB,)),
                pltpu.SemaphoreType.DMA((3 * NG,)),
                pltpu.SemaphoreType.DMA((4,)),
                pltpu.SemaphoreType.DMA((NB,)),
                pltpu.SemaphoreType.DMA((2,)),
            ],
            compiler_params=pltpu.CompilerParams(vmem_limit_bytes=110 * 1024 * 1024),
        )(A_x.reshape(S, D), A_wqkv, A_wo, B_w1, B_b1, B_w2, B_b2)
        return out.reshape(1, S, D)

    return run


@jax.jit
def pallas_interleave_layers__sliding_local_dilated__dense_activation_squared_relu__prompt_kernel(A_x, A_wqkv, A_wo, B_x, B_w1, B_b1, B_w2, B_b2):
    return make()(A_x, A_wqkv, A_wo, B_x, B_w1, B_b1, B_w2, B_b2)
```

```python
import functools
import numpy as np
import jax
import jax.numpy as jnp
from jax import lax
import jax.experimental.pallas as pl
import jax.experimental.pallas.tpu as pltpu

S, D, F, H, DH = 2048, 1024, 3584, 32, 32
WIN, DIL = 8, 2
EPS = 1e-5
F32, BF16, U32 = jnp.float32, jnp.bfloat16, jnp.uint32

NN = (((1,), (0,)), ((), ()))


def _dot(a, b, dims=NN):
    return lax.dot_general(a, b, dims, preferred_element_type=F32)


def _ln(x):
    m = jnp.mean(x, axis=-1, keepdims=True)
    c = x - m
    v = jnp.mean(c * c, axis=-1, keepdims=True)
    return c * lax.rsqrt(v + EPS)


def _unpack(w):
    lo = pltpu.unpack_elementwise(w, index=0, packed_dtype=BF16, unpacked_dtype=F32)
    hi = pltpu.unpack_elementwise(w, index=1, packed_dtype=BF16, unpacked_dtype=F32)
    return lo, hi


def _pk(x):
    return pltpu.bitcast(x.astype(BF16), U32)


def _bf(w):
    return pltpu.bitcast(w, BF16)


def make(R=256, LNC=16, LNB=32, NL=2, WOS=4, WAITS=(0, 1, 2, 3, 4, 5, 6, 7), AHEAD=9, AF=(0, 1), DEFER=1,
         SCOPES=False, ONLY=None, LNP=1):
    NB = S // R
    assert R == 256
    GR = 128
    NG = D // GR
    NH = DH // 8
    GP = GR // 2
    XN0 = S + R
    QX0 = 3 * D
    NQ = D // 128

    def scoped(name, fn):
        if SCOPES:
            with jax.named_scope(name):
                fn()
        else:
            fn()

    def kernel(x_hbm, wqkv_hbm, wo_hbm, w1_hbm, b1_ref, w2_hbm, b2_ref, out_hbm,
               xin, wqkv, wo, w1, w2, bb1, bb2, xa, xb, qkv, qkv0, kprev, vprev, o, h, ostage,
               sem_x, sem_qkv, sem_w, sem_o, sem_c):
        cp_q = [[pltpu.make_async_copy(wqkv_hbm.at[:, pl.ds(p * D + g * GR, GR)],
                                       wqkv.at[:, pl.ds(p * D + g * GR, GR)],
                                       sem_qkv.at[g * 3 + p]) for p in range(3)] for g in range(NG)]

        def rows(r, n):
            return pl.ds(r if isinstance(r, int) else pl.multiple_of(r, n), n)

        def blk(i):
            return rows(i * R, R)

        def cp_x(i):
            return pltpu.make_async_copy(x_hbm.at[blk(i)], xin.at[blk(i)], sem_x.at[i])

        def cp_o(i):
            return pltpu.make_async_copy(ostage.at[blk(i)], out_hbm.at[blk(i)], sem_o.at[i])

        cp_ba = pltpu.make_async_copy(xb.at[blk(0)], xa.at[blk(NB)], sem_c.at[0])
        cp_ab = pltpu.make_async_copy(xa.at[blk(0)], xb.at[blk(NB)], sem_c.at[1])

        k1 = WOS * GR
        cp_wo1 = pltpu.make_async_copy(wo_hbm.at[:k1], wo.at[:k1], sem_w.at[0])
        cp_wo2 = pltpu.make_async_copy(wo_hbm.at[k1:], wo.at[k1:], sem_w.at[3])
        cp_w1 = pltpu.make_async_copy(w1_hbm, w1, sem_w.at[1])
        cp_w2 = pltpu.make_async_copy(w2_hbm, w2, sem_w.at[2])

        queue = [[cp_x(0)]] + cp_q + [[cp_wo1], [cp_x(1), cp_wo2]]
        issued = [0]

        def issue(n):
            while issued[0] < min(n, len(queue)):
                for c in queue[issued[0]]:
                    c.start()
                issued[0] += 1

        issue(2)

        bb1[...] = jnp.broadcast_to(b1_ref[...].astype(F32).reshape(1, F), (8, F))
        bb2[...] = jnp.broadcast_to(b2_ref[...].astype(F32).reshape(1, D), (8, D))

        def get_xn():
            return pltpu.bitcast(xb[pl.ds(XN0, R // 2), :], BF16)

        def load_x(src_ref, i, off, n, from_input):
            sl = rows(i * R + off, n)
            if from_input is False:
                return src_ref[sl, :]
            if from_input is True:
                return xin[sl, :].astype(F32)
            si = rows(jnp.minimum(i, NB - 1) * R + off, n)
            return jnp.where(from_input, xin[si, :].astype(F32), src_ref[sl, :])

        def layernorm(src_ref, i, from_input=False, zero=0):
            for c in range(R // LNB):
                y = _ln(load_x(src_ref, i, c * LNB, LNB, from_input))
                xb[rows(zero + XN0 + c * LNB // 2, LNB // 2), :] = pltpu.bitcast(y.astype(BF16), F32)

        def layernorm_staged(i, zero, from_input):
            for c in range(R // LNC):
                y = _pk(_ln(load_x(xa, i, c * LNC, LNC, from_input)))
                for k in range(NQ):
                    qkv[rows(zero + QX0 + k * (R // 2) + c * LNC // 2, LNC // 2), :] = y[:, k * 128:(k + 1) * 128]

        def unstage():
            for k in range(NQ):
                xb[pl.ds(XN0, R // 2), pl.ds(k * 128, 128)] = pltpu.bitcast(
                    qkv[pl.ds(QX0 + k * (R // 2), R // 2), :], F32)

        lane = lax.broadcasted_iota(jnp.int32, (8, 128), 1)
        sub = lax.broadcasted_iota(jnp.int32, (8, 128), 0)
        m_even = (sub & 2) == 0
        m_odd = ((sub + 7) & 2) == 0
        m_par = (sub & 1) == 0

        def attention(g, first):
            base = g * 3 * GR

            def shifted(part, prev_ref, d):
                cur = qkv[pl.ds(base + part * GR + d * 8, 8), :]
                out = [_unpack(cur)]
                if first is True or part == 2:
                    b = jnp.broadcast_to(out[0][0][:, 0:1], (8, 128))
                    prev = pltpu.pack_elementwise([b, b], packed_dtype=BF16)
                if first is not True:
                    old = prev_ref[pl.ds(g * GR + d * 8, 8), :]
                    prev = jnp.where(first, prev, old) if part == 2 else old
                for w in range(1, WIN):
                    out.append(_unpack(pltpu.roll(jnp.where(lane >= 128 - w, prev, cur), w, 1)))
                return out

            outs = []
            for hp in range(GR // DH // 2):
                half = []
                for hd in (2 * hp, 2 * hp + 1):
                    acc = [[None, None] for _ in range(WIN)]
                    for d in range(hd * NH, (hd + 1) * NH):
                        q = _unpack(qkv[pl.ds(base + d * 8, 8), :])
                        ks = shifted(1, kprev, d)
                        for w in range(WIN):
                            for k in range(2):
                                pr = q[k] * ks[w][k]
                                acc[w][k] = pr if acc[w][k] is None else acc[w][k] + pr
                    m = m_odd if hd % 2 else m_even
                    half.append([jnp.where(m, a, b) + pltpu.roll(jnp.where(m, b, a), 6, 0) for a, b in acc])
                lg = []
                for u, v in zip(*half):
                    z = jnp.where(m_par, u, v) + pltpu.roll(jnp.where(m_par, v, u), 7, 0)
                    lg.append((z + pltpu.roll(z, 4, 0)) * (DH ** -0.5))
                lg = [lg[0]] + [jnp.where(jnp.logical_and(first, lane < w), -1e9, lg[w]) for w in range(1, WIN)]
                mx = functools.reduce(jnp.maximum, lg)
                e = [jnp.exp(a - mx) for a in lg]
                inv = 1.0 / functools.reduce(jnp.add, e)
                p = [a * inv for a in e]
                for hd in (2 * hp, 2 * hp + 1):
                    ph = [[jnp.broadcast_to(a[hd % 2 + 2 * k:hd % 2 + 2 * k + 1, :], (8, 128)) for k in range(2)]
                          for a in p]
                    for d in range(hd * NH, (hd + 1) * NH):
                        vs = shifted(2, vprev, d)
                        os_ = []
                        for k in range(2):
                            acc_o = ph[0][k] * vs[0][k]
                            for w in range(1, WIN):
                                acc_o = acc_o + ph[w][k] * vs[w][k]
                            os_.append(acc_o)
                        outs.append(pltpu.pack_elementwise(os_, packed_dtype=BF16))
            o[:, pl.ds(g * GR, GR)] = jnp.concatenate(outs, axis=0).T
            kprev[pl.ds(g * GR, GR), :] = qkv[pl.ds(base + GR, GR), :]
            vprev[pl.ds(g * GR, GR), :] = qkv[pl.ds(base + 2 * GR, GR), :]

        def fold(a):
            u = jnp.where(m_even, a[0], a[2]) + pltpu.roll(jnp.where(m_even, a[2], a[0]), 6, 0)
            v = jnp.where(m_odd, a[1], a[3]) + pltpu.roll(jnp.where(m_odd, a[3], a[1]), 6, 0)
            z = jnp.where(m_par, u, v) + pltpu.roll(jnp.where(m_par, v, u), 7, 0)
            return z + pltpu.roll(z, 4, 0)

        def attention_first(g):
            base = g * 3 * GP
            for t in range(R // 128):
                cols = pl.ds(t * 128, 128)

                def shifted(part, d):
                    rs = pl.ds(base + part * GP + d * 8, 8)
                    cur = qkv0[rs, cols]
                    if t == 0:
                        prev = jnp.broadcast_to(cur[:, 0:1], (8, 128))
                    else:
                        prev = qkv0[rs, pl.ds((t - 1) * 128, 128)]
                    out = [_unpack(cur)]
                    for w in range(1, WIN):
                        sh = w * DIL
                        out.append(_unpack(pltpu.roll(jnp.where(lane >= 128 - sh, prev, cur), sh, 1)))
                    return out

                acc = [[None] * 4 for _ in range(WIN)]
                for d in range(GP // 8):
                    hd = d // 2
                    q0, q1 = _unpack(qkv0[pl.ds(base + d * 8, 8), cols])
                    ks = shifted(1, d)
                    for w in range(WIN):
                        pr = q0 * ks[w][0] + q1 * ks[w][1]
                        acc[w][hd] = pr if acc[w][hd] is None else acc[w][hd] + pr
                lg = [fold(a) * (DH ** -0.5) for a in acc]
                if t == 0:
                    lg = [lg[0]] + [jnp.where(lane < w * DIL, -1e9, lg[w])
                                    for w in range(1, WIN)]
                m = functools.reduce(jnp.maximum, lg)
                e = [jnp.exp(a - m) for a in lg]
                inv = 1.0 / functools.reduce(jnp.add, e)
                p = [a * inv for a in e]
                outs = []
                for d in range(GP // 8):
                    hd = d // 2
                    if d % 2 == 0:
                        ph = [jnp.broadcast_to(a[hd:hd + 1, :], (8, 128)) for a in p]
                    vs = shifted(2, d)
                    os_ = []
                    for k in range(2):
                        acc_o = ph[0] * vs[0][k]
                        for w in range(1, WIN):
                            acc_o = acc_o + ph[w] * vs[w][k]
                        os_.append(acc_o)
                    outs.append(_bf(pltpu.pack_elementwise(os_, packed_dtype=BF16)))
                oT = jnp.concatenate(outs, axis=0)
                o[pl.ds(t * 64, 64), pl.ds(g * GR, GR)] = pltpu.bitcast(oT.T, U32)

        def attn_unit(i, l, peeled=False):
            first = True if peeled else i == 0
            waited = [0]
            pending = []

            def flush():
                while pending:
                    g, p = pending.pop(0)
                    qkv0[pl.ds((g * 3 + p) * GP, GP), :] = pltpu.bitcast(_bf(vprev[pl.ds(g * GR, GR), :]).T, U32)

            def need(g):
                if peeled and waited[0] <= g < NG:
                    nxt = min([w for w in WAITS if w > g] + [NG])
                    issue(nxt + 1)
                    for gg in range(waited[0], nxt):
                        scoped(f"wq{gg}", lambda: [c.wait() for c in cp_q[gg]] and None)
                    issue(nxt + 1 + AHEAD)
                    waited[0] = nxt
                    flush()

            def proj(g):
                need(g)
                for p in range(3):
                    if g == 0 and p == LNP and not peeled:
                        layernorm_staged(i + 1, i >> 8, jnp.logical_and(l == 0, i + 1 < NB))
                    y = _pk(_dot(get_xn(), wqkv[:, pl.ds(p * D + g * GR, GR)]))
                    if not peeled:
                        qkv[pl.ds((g * 3 + p) * GR, GR), :] = y.T
                        continue
                    if p:
                        (kprev, vprev)[p - 1][pl.ds(g * GR, GR), :] = y
                    if p == 2 and (g + 1 in WAITS or g + 1 == NG):
                        pending.append((g, p))
                    else:
                        qkv0[pl.ds((g * 3 + p) * GP, GP), :] = pltpu.bitcast(_bf(y).T, U32)

            def attend(g):
                if peeled:
                    attention_first(g)
                else:
                    attention(g, first)

            proj(0)
            for g in range(NG - 1):
                if AF[int(peeled)]:
                    need(g + 1)
                    attend(g)
                    proj(g + 1)
                else:
                    proj(g + 1)
                    attend(g)
            if peeled:
                issue(len(queue))
                scoped("wwo1", cp_wo1.wait)
                for j in range(2, NB):
                    cp_x(j).start()
                flush()
            y = _dot(_bf(o[:, :k1]), wo[:k1, :])
            xb[blk(i), :] = load_x(xa, i, 0, R, True if peeled else l == 0) + y
            attend(NG - 1)
            if peeled:
                scoped("wx1", cp_x(1).wait)
                scoped("wwo2", cp_wo2.wait)
                cp_w1.start()
                cp_w2.start()
                layernorm(xa, 1, True, pl.program_id(0))
                for g in range(NG):
                    for ref in (kprev, vprev):
                        ref[pl.ds(g * GR, GR), :] = ref[pl.ds(g * GR, GR), :].T
            else:
                unstage()
            y = _dot(_bf(o[:, k1:]), wo[k1:, :])
            xb[blk(i), :] = xb[blk(i), :] + y

        def ffn_unit(i):
            hh = _dot(get_xn(), w1[...]) + bb1[0:1, :]
            rr = jnp.where(hh > 0, hh, 0.0)
            h[...] = _pk(rr * rr)
            layernorm(xb, i + 1)
            x2 = xb[blk(i), :] + (_dot(_bf(h[...]), w2[...]) + bb2[0:1, :])
            xa[blk(i), :] = x2
            ostage[blk(i), :] = x2.astype(BF16)

        scoped("wait_x0", lambda: cp_x(0).wait())
        issue(1 + AHEAD)
        layernorm(xa, 0, True)
        if ONLY in (None, "P"):
            scoped("attn_first", lambda: attn_unit(0, 0, True))

        def layer(l, carry):
            def _a(i, c):
                @pl.when(jnp.logical_and(l == 0, i + 1 < NB))
                def _():
                    cp_x(i + 1).wait()

                @pl.when(i == 1)
                def _():
                    cp_ba.start()

                @pl.when(i == NB - 1)
                def _():
                    cp_ba.wait()

                scoped("attn_unit", lambda: attn_unit(i, l))
                return c
            if ONLY in (None, "A"):
                lax.fori_loop(jnp.where(l == 0, 1, 0), NB, _a, 0)

            @pl.when(l == 0)
            def _():
                cp_w1.wait()
                cp_w2.wait()

            def _b(i, c):
                @pl.when(i == 1)
                def _():
                    cp_ab.start()

                @pl.when(i == NB - 1)
                def _():
                    cp_ab.wait()

                scoped("ffn_unit", lambda: ffn_unit(i))

                @pl.when(l == NL - 1)
                def _():
                    cp_o(i).start()
                return c
            if ONLY in (None, "B"):
                lax.fori_loop(0, NB, _b, 0)
            return carry

        lax.fori_loop(0, NL, layer, 0)
        for i in range(NB):
            cp_o(i).wait()

    def run(A_x, A_wqkv, A_wo, B_x, B_w1, B_b1, B_w2, B_b2):
        del B_x
        hbm = pl.BlockSpec(memory_space=pl.ANY)
        vm = pl.BlockSpec(memory_space=pltpu.VMEM)
        out = pl.pallas_call(
            kernel,
            out_shape=jax.ShapeDtypeStruct((S, D), BF16),
            grid=(1,),
            in_specs=[hbm, hbm, hbm, hbm, vm, hbm, vm],
            out_specs=hbm,
            scratch_shapes=[
                pltpu.VMEM((S, D), BF16),
                pltpu.VMEM((D, 3 * D), BF16),
                pltpu.VMEM((D, D), BF16),
                pltpu.VMEM((D, F), BF16),
                pltpu.VMEM((F, D), BF16),
                pltpu.VMEM((8, F), F32),
                pltpu.VMEM((8, D), F32),
                pltpu.VMEM((S + R, D), F32),
                pltpu.VMEM((S + R + R // 2, D), F32),
                pltpu.VMEM((4 * D, 128), U32),
                pltpu.VMEM((3 * D // 2, R), U32),
                pltpu.VMEM((D, 128), U32),
                pltpu.VMEM((D, 128), U32),
                pltpu.VMEM((R // 2, D), U32),
                pltpu.VMEM((R // 2, F), U32),
                pltpu.VMEM((S, D), BF16),
                pltpu.SemaphoreType.DMA((NB,)),
                pltpu.SemaphoreType.DMA((3 * NG,)),
                pltpu.SemaphoreType.DMA((4,)),
                pltpu.SemaphoreType.DMA((NB,)),
                pltpu.SemaphoreType.DMA((2,)),
            ],
            compiler_params=pltpu.CompilerParams(vmem_limit_bytes=110 * 1024 * 1024),
        )(A_x.reshape(S, D), A_wqkv, A_wo, B_w1, B_b1, B_w2, B_b2)
        return out.reshape(1, S, D)

    return run


@jax.jit
def pallas_interleave_layers__sliding_local_dilated__dense_activation_squared_relu__prompt_kernel(A_x, A_wqkv, A_wo, B_x, B_w1, B_b1, B_w2, B_b2):
    return make(WOS=5,LNP=0,LNC=32)(A_x, A_wqkv, A_wo, B_x, B_w1, B_b1, B_w2, B_b2)
```

```python
import functools
import numpy as np
import jax
import jax.numpy as jnp
from jax import lax
import jax.experimental.pallas as pl
import jax.experimental.pallas.tpu as pltpu

S, D, F, H, DH = 2048, 1024, 3584, 32, 32
WIN, DIL = 8, 2
EPS = 1e-5
F32, BF16, U32 = jnp.float32, jnp.bfloat16, jnp.uint32

NN = (((1,), (0,)), ((), ()))


def _dot(a, b, dims=NN):
    return lax.dot_general(a, b, dims, preferred_element_type=F32)


def _ln(x):
    m = jnp.mean(x, axis=-1, keepdims=True)
    c = x - m
    v = jnp.mean(c * c, axis=-1, keepdims=True)
    return c * lax.rsqrt(v + EPS)


def _unpack(w):
    lo = pltpu.unpack_elementwise(w, index=0, packed_dtype=BF16, unpacked_dtype=F32)
    hi = pltpu.unpack_elementwise(w, index=1, packed_dtype=BF16, unpacked_dtype=F32)
    return lo, hi


def _pk(x):
    return pltpu.bitcast(x.astype(BF16), U32)


def _bf(w):
    return pltpu.bitcast(w, BF16)


def make(R=256, LNC=32, LNB=32, NL=2, WOS=5, WAITS=(0, 1, 2, 3, 4, 5, 6, 7), AHEAD=9, AF=(0, 1), DEFER=1,
         SCOPES=False, W32=1, UNS=1, HALO=0, EX2=0, QKF=0, KO=(0, 1, 2), WC=0, ONLY=None, LNP=0):
    NB = S // R
    assert R == 256
    GR = 128
    NG = D // GR
    NH = DH // 8
    GP = GR // 2
    XN0 = S + R
    QX0 = 3 * D
    NQ = D // 128

    def scoped(name, fn):
        if SCOPES:
            with jax.named_scope(name):
                fn()
        else:
            fn()

    def kernel(x_hbm, wqkv_hbm, wo_hbm, w1_hbm, b1_ref, w2_hbm, b2_ref, out_hbm,
               xin, wqkv, wo, wq32, wo32, w1, w2, bb1, bb2, xa, xb, qkv, qkv0, kprev, vprev, o, h, ostage,
               sem_x, sem_qkv, sem_w, sem_o, sem_c):
        cp_q = [[pltpu.make_async_copy(wqkv_hbm.at[:, pl.ds(p * D + g * GR, GR)],
                                       wqkv.at[:, pl.ds(p * D + g * GR, GR)],
                                       sem_qkv.at[g * 3 + p]) for p in range(3)] for g in range(NG)]

        def rows(r, n):
            return pl.ds(r if isinstance(r, int) else pl.multiple_of(r, n), n)

        def blk(i):
            return rows(i * R, R)

        def cp_x(i):
            return pltpu.make_async_copy(x_hbm.at[blk(i)], xin.at[blk(i)], sem_x.at[i])

        def cp_o(i):
            return pltpu.make_async_copy(ostage.at[blk(i)], out_hbm.at[blk(i)], sem_o.at[i])

        cp_ba = pltpu.make_async_copy(xb.at[blk(0)], xa.at[blk(NB)], sem_c.at[0])
        cp_ab = pltpu.make_async_copy(xa.at[blk(0)], xb.at[blk(NB)], sem_c.at[1])

        k1 = WOS * GR
        cp_wo1 = pltpu.make_async_copy(wo_hbm.at[:k1], wo.at[:k1], sem_w.at[0])
        cp_wo2 = pltpu.make_async_copy(wo_hbm.at[k1:], wo.at[k1:], sem_w.at[3])
        cp_w1 = pltpu.make_async_copy(w1_hbm, w1, sem_w.at[1])
        cp_w2 = pltpu.make_async_copy(w2_hbm, w2, sem_w.at[2])

        queue = [[cp_x(0)]] + cp_q + [[cp_wo1], [cp_x(1), cp_wo2]]
        issued = [0]

        def issue(n):
            while issued[0] < min(n, len(queue)):
                for c in queue[issued[0]]:
                    c.start()
                issued[0] += 1

        issue(2)

        bb1[...] = jnp.broadcast_to(b1_ref[...].astype(F32).reshape(1, F), (8, F))
        bb2[...] = jnp.broadcast_to(b2_ref[...].astype(F32).reshape(1, D), (8, D))

        def get_xn():
            return pltpu.bitcast(xb[pl.ds(XN0, R // 2), :], BF16)

        def load_x(src_ref, i, off, n, from_input):
            sl = rows(i * R + off, n)
            if from_input is False:
                return src_ref[sl, :]
            if from_input is True:
                return xin[sl, :].astype(F32)
            si = rows(jnp.minimum(i, NB - 1) * R + off, n)
            return jnp.where(from_input, xin[si, :].astype(F32), src_ref[sl, :])

        def layernorm(src_ref, i, from_input=False, zero=0):
            for c in range(R // LNB):
                y = _ln(load_x(src_ref, i, c * LNB, LNB, from_input))
                xb[rows(zero + XN0 + c * LNB // 2, LNB // 2), :] = pltpu.bitcast(y.astype(BF16), F32)

        def layernorm_staged(i, zero, from_input):
            for c in range(R // LNC):
                y = _pk(_ln(load_x(xa, i, c * LNC, LNC, from_input)))
                for k in range(NQ):
                    qkv[rows(zero + QX0 + k * (R // 2) + c * LNC // 2, LNC // 2), :] = y[:, k * 128:(k + 1) * 128]

        def unstage():
            for k in range(NQ):
                xb[pl.ds(XN0, R // 2), pl.ds(k * 128, 128)] = pltpu.bitcast(
                    qkv[pl.ds(QX0 + k * (R // 2), R // 2), :], F32)

        lane = lax.broadcasted_iota(jnp.int32, (8, 128), 1)
        sub = lax.broadcasted_iota(jnp.int32, (8, 128), 0)
        m_even = (sub & 2) == 0
        m_odd = ((sub + 7) & 2) == 0
        m_par = (sub & 1) == 0

        def attention(g, first):
            base = g * 3 * GR

            def shifted(part, prev_ref, d):
                cur = qkv[pl.ds(base + part * GR + d * 8, 8), :]
                out = [_unpack(cur)]
                if first is True or part == 2:
                    b = jnp.broadcast_to(out[0][0][:, 0:1], (8, 128))
                    prev = pltpu.pack_elementwise([b, b], packed_dtype=BF16)
                if first is not True:
                    old = prev_ref[pl.ds(g * GR + d * 8, 8), :]
                    prev = jnp.where(first, prev, old) if part == 2 else old
                for w in range(1, WIN):
                    out.append(_unpack(pltpu.roll(jnp.where(lane >= 128 - w, prev, cur), w, 1)))
                return out

            def probs(hp):
                half = []
                for hd in (2 * hp, 2 * hp + 1):
                    acc = [[None, None] for _ in range(WIN)]
                    for d in range(hd * NH, (hd + 1) * NH):
                        q = _unpack(qkv[pl.ds(base + d * 8, 8), :])
                        ks = shifted(1, kprev, d)
                        for w in range(WIN):
                            for k in range(2):
                                pr = q[k] * ks[w][k]
                                acc[w][k] = pr if acc[w][k] is None else acc[w][k] + pr
                    m = m_odd if hd % 2 else m_even
                    half.append([jnp.where(m, a, b) + pltpu.roll(jnp.where(m, b, a), 6, 0) for a, b in acc])
                lg = []
                for u, v in zip(*half):
                    z = jnp.where(m_par, u, v) + pltpu.roll(jnp.where(m_par, v, u), 7, 0)
                    lg.append((z + pltpu.roll(z, 4, 0)) * (DH ** -0.5))
                lg = [lg[0]] + [jnp.where(jnp.logical_and(first, lane < w), -1e9, lg[w]) for w in range(1, WIN)]
                mx = functools.reduce(jnp.maximum, lg)
                e = [jnp.exp(a - mx) for a in lg]
                inv = 1.0 / functools.reduce(jnp.add, e)
                return [a * inv for a in e]

            def values(hp, p):
                outs = []
                for hd in (2 * hp, 2 * hp + 1):
                    ph = [[jnp.broadcast_to(a[hd % 2 + 2 * k:hd % 2 + 2 * k + 1, :], (8, 128)) for k in range(2)]
                          for a in p]
                    for d in range(hd * NH, (hd + 1) * NH):
                        vs = shifted(2, vprev, d)
                        os_ = []
                        for k in range(2):
                            if EX2:
                                t = [ph[w][k] * vs[w][k] for w in range(WIN)]
                                acc_o = ((t[0] + t[1]) + (t[2] + t[3])) + ((t[4] + t[5]) + (t[6] + t[7]))
                            else:
                                acc_o = ph[0][k] * vs[0][k]
                                for w in range(1, WIN):
                                    acc_o = acc_o + ph[w][k] * vs[w][k]
                            os_.append(acc_o)
                        outs.append(pltpu.pack_elementwise(os_, packed_dtype=BF16))
                return outs

            if QKF:
                ps = [probs(0), probs(1)]
                outs = values(0, ps[0]) + values(1, ps[1])
            else:
                outs = values(0, probs(0)) + values(1, probs(1))
            o[:, pl.ds(g * GR, GR)] = jnp.concatenate(outs, axis=0).T
            if HALO == 0:
                save_halo(g)

        def save_halo(g):
            kprev[pl.ds(g * GR, GR), :] = qkv[pl.ds((g * 3 + 1) * GR, GR), :]
            vprev[pl.ds(g * GR, GR), :] = qkv[pl.ds((g * 3 + 2) * GR, GR), :]

        def fold(a):
            u = jnp.where(m_even, a[0], a[2]) + pltpu.roll(jnp.where(m_even, a[2], a[0]), 6, 0)
            v = jnp.where(m_odd, a[1], a[3]) + pltpu.roll(jnp.where(m_odd, a[3], a[1]), 6, 0)
            z = jnp.where(m_par, u, v) + pltpu.roll(jnp.where(m_par, v, u), 7, 0)
            return z + pltpu.roll(z, 4, 0)

        def attention_first(g):
            base = g * 3 * GP
            for t in range(R // 128):
                cols = pl.ds(t * 128, 128)

                def shifted(part, d):
                    rs = pl.ds(base + part * GP + d * 8, 8)
                    cur = qkv0[rs, cols]
                    if t == 0:
                        prev = jnp.broadcast_to(cur[:, 0:1], (8, 128))
                    else:
                        prev = qkv0[rs, pl.ds((t - 1) * 128, 128)]
                    out = [_unpack(cur)]
                    for w in range(1, WIN):
                        sh = w * DIL
                        out.append(_unpack(pltpu.roll(jnp.where(lane >= 128 - sh, prev, cur), sh, 1)))
                    return out

                acc = [[None] * 4 for _ in range(WIN)]
                for d in range(GP // 8):
                    hd = d // 2
                    q0, q1 = _unpack(qkv0[pl.ds(base + d * 8, 8), cols])
                    ks = shifted(1, d)
                    for w in range(WIN):
                        pr = q0 * ks[w][0] + q1 * ks[w][1]
                        acc[w][hd] = pr if acc[w][hd] is None else acc[w][hd] + pr
                lg = [fold(a) * (DH ** -0.5) for a in acc]
                if t == 0:
                    lg = [lg[0]] + [jnp.where(lane < w * DIL, -1e9, lg[w])
                                    for w in range(1, WIN)]
                m = functools.reduce(jnp.maximum, lg)
                e = [jnp.exp(a - m) for a in lg]
                inv = 1.0 / functools.reduce(jnp.add, e)
                p = [a * inv for a in e]
                outs = []
                for d in range(GP // 8):
                    hd = d // 2
                    if d % 2 == 0:
                        ph = [jnp.broadcast_to(a[hd:hd + 1, :], (8, 128)) for a in p]
                    vs = shifted(2, d)
                    os_ = []
                    for k in range(2):
                        acc_o = ph[0] * vs[0][k]
                        for w in range(1, WIN):
                            acc_o = acc_o + ph[w] * vs[w][k]
                        os_.append(acc_o)
                    outs.append(_bf(pltpu.pack_elementwise(os_, packed_dtype=BF16)))
                oT = jnp.concatenate(outs, axis=0)
                o[pl.ds(t * 64, 64), pl.ds(g * GR, GR)] = pltpu.bitcast(oT.T, U32)

        def attn_unit(i, l, peeled=False):
            first = True if peeled else i == 0
            waited = [0]
            pending = []

            def flush():
                while pending:
                    g, p = pending.pop(0)
                    qkv0[pl.ds((g * 3 + p) * GP, GP), :] = pltpu.bitcast(_bf(vprev[pl.ds(g * GR, GR), :]).T, U32)

            def need(g):
                if peeled and waited[0] <= g < NG:
                    nxt = min([w for w in WAITS if w > g] + [NG])
                    issue(nxt + 1)
                    for gg in range(waited[0], nxt):
                        scoped(f"wq{gg}", lambda: [c.wait() for c in cp_q[gg]] and None)
                    issue(nxt + 1 + AHEAD)
                    waited[0] = nxt
                    flush()

            def proj(g):
                need(g)
                for n, p in enumerate((0, 1, 2) if peeled else KO):
                    if g == 0 and n == LNP and not peeled:
                        layernorm_staged(i + 1, i >> 8, jnp.logical_and(l == 0, i + 1 < NB))
                    cs = pl.ds(p * D + g * GR, GR)
                    if W32 and not peeled:
                        wv = _bf(wq32[:, cs])
                    else:
                        wv = wqkv[:, cs]
                        if W32:
                            wq32[:, cs] = pltpu.bitcast(wv, U32)
                    y = _pk(_dot(get_xn(), wv))
                    if not peeled:
                        qkv[pl.ds((g * 3 + p) * GR, GR), :] = y.T
                        continue
                    if p:
                        (kprev, vprev)[p - 1][pl.ds(g * GR, GR), :] = y
                    if p == 2 and (g + 1 in WAITS or g + 1 == NG):
                        pending.append((g, p))
                    else:
                        qkv0[pl.ds((g * 3 + p) * GP, GP), :] = pltpu.bitcast(_bf(y).T, U32)

            def attend(g):
                if peeled:
                    attention_first(g)
                else:
                    attention(g, first)

            proj(0)
            for g in range(NG - 1):
                if AF[int(peeled)]:
                    need(g + 1)
                    attend(g)
                    proj(g + 1)
                else:
                    proj(g + 1)
                    attend(g)
            if peeled:
                issue(len(queue))
                scoped("wwo1", cp_wo1.wait)
                for j in range(2, NB):
                    cp_x(j).start()
                flush()
            if UNS == 0 and not peeled:
                unstage()

            def get_wo(a, b, cs):
                if W32 == 2 and not peeled:
                    return _bf(wo32[a // 2:b // 2, cs])
                wv = wo[a:b, cs]
                if W32 == 2:
                    wo32[a // 2:b // 2, cs] = pltpu.bitcast(wv, U32)
                return wv

            y = _dot(_bf(o[:, :k1]), get_wo(0, k1, slice(None)))
            xb[blk(i), :] = load_x(xa, i, 0, R, True if peeled else l == 0) + y
            attend(NG - 1)
            if peeled:
                scoped("wx1", cp_x(1).wait)
                scoped("wwo2", cp_wo2.wait)
                cp_w1.start()
                cp_w2.start()
                layernorm(xa, 1, True, pl.program_id(0))
                for g in range(NG):
                    for ref in (kprev, vprev):
                        ref[pl.ds(g * GR, GR), :] = ref[pl.ds(g * GR, GR), :].T
            elif UNS == 1:
                unstage()
            if HALO and not peeled:
                for g in range(NG):
                    save_halo(g)
            nc = D // WC if WC else D
            for c in range(0, D, nc):
                cs = pl.ds(c, nc)
                xb[blk(i), cs] = xb[blk(i), cs] + _dot(_bf(o[:, k1:]), get_wo(k1, D, cs))

        def ffn_unit(i):
            hh = _dot(get_xn(), w1[...]) + bb1[0:1, :]
            rr = jnp.where(hh > 0, hh, 0.0)
            h[...] = _pk(rr * rr)
            layernorm(xb, i + 1)
            x2 = xb[blk(i), :] + (_dot(_bf(h[...]), w2[...]) + bb2[0:1, :])
            xa[blk(i), :] = x2
            ostage[blk(i), :] = x2.astype(BF16)

        scoped("wait_x0", lambda: cp_x(0).wait())
        issue(1 + AHEAD)
        layernorm(xa, 0, True)
        if ONLY in (None, "P"):
            scoped("attn_first", lambda: attn_unit(0, 0, True))

        def layer(l, carry):
            def _a(i, c):
                @pl.when(jnp.logical_and(l == 0, i + 1 < NB))
                def _():
                    cp_x(i + 1).wait()

                @pl.when(i == 1)
                def _():
                    cp_ba.start()

                @pl.when(i == NB - 1)
                def _():
                    cp_ba.wait()

                scoped("attn_unit", lambda: attn_unit(i, l))
                return c
            if ONLY in (None, "A"):
                lax.fori_loop(jnp.where(l == 0, 1, 0), NB, _a, 0)

            @pl.when(l == 0)
            def _():
                cp_w1.wait()
                cp_w2.wait()

            def _b(i, c):
                @pl.when(i == 1)
                def _():
                    cp_ab.start()

                @pl.when(i == NB - 1)
                def _():
                    cp_ab.wait()

                scoped("ffn_unit", lambda: ffn_unit(i))

                @pl.when(l == NL - 1)
                def _():
                    cp_o(i).start()
                return c
            if ONLY in (None, "B"):
                lax.fori_loop(0, NB, _b, 0)
            return carry

        lax.fori_loop(0, NL, layer, 0)
        for i in range(NB):
            cp_o(i).wait()

    def run(A_x, A_wqkv, A_wo, B_x, B_w1, B_b1, B_w2, B_b2):
        del B_x
        hbm = pl.BlockSpec(memory_space=pl.ANY)
        vm = pl.BlockSpec(memory_space=pltpu.VMEM)
        out = pl.pallas_call(
            kernel,
            out_shape=jax.ShapeDtypeStruct((S, D), BF16),
            grid=(1,),
            in_specs=[hbm, hbm, hbm, hbm, vm, hbm, vm],
            out_specs=hbm,
            scratch_shapes=[
                pltpu.VMEM((S, D), BF16),
                pltpu.VMEM((D, 3 * D), BF16),
                pltpu.VMEM((D, D), BF16),
                pltpu.VMEM((D // 2, 3 * D), U32),
                pltpu.VMEM((D // 2, D), U32),
                pltpu.VMEM((D, F), BF16),
                pltpu.VMEM((F, D), BF16),
                pltpu.VMEM((8, F), F32),
                pltpu.VMEM((8, D), F32),
                pltpu.VMEM((S + R, D), F32),
                pltpu.VMEM((S + R + R // 2, D), F32),
                pltpu.VMEM((4 * D, 128), U32),
                pltpu.VMEM((3 * D // 2, R), U32),
                pltpu.VMEM((D, 128), U32),
                pltpu.VMEM((D, 128), U32),
                pltpu.VMEM((R // 2, D), U32),
                pltpu.VMEM((R // 2, F), U32),
                pltpu.VMEM((S, D), BF16),
                pltpu.SemaphoreType.DMA((NB,)),
                pltpu.SemaphoreType.DMA((3 * NG,)),
                pltpu.SemaphoreType.DMA((4,)),
                pltpu.SemaphoreType.DMA((NB,)),
                pltpu.SemaphoreType.DMA((2,)),
            ],
            compiler_params=pltpu.CompilerParams(vmem_limit_bytes=110 * 1024 * 1024),
        )(A_x.reshape(S, D), A_wqkv, A_wo, B_w1, B_b1, B_w2, B_b2)
        return out.reshape(1, S, D)

    return run


@jax.jit
def pallas_interleave_layers__sliding_local_dilated__dense_activation_squared_relu__prompt_kernel(A_x, A_wqkv, A_wo, B_x, B_w1, B_b1, B_w2, B_b2):
    return make(W32=1)(A_x, A_wqkv, A_wo, B_x, B_w1, B_b1, B_w2, B_b2)
```

```python
import functools
import numpy as np
import jax
import jax.numpy as jnp
from jax import lax
import jax.experimental.pallas as pl
import jax.experimental.pallas.tpu as pltpu

S, D, F, H, DH = 2048, 1024, 3584, 32, 32
WIN, DIL = 8, 2
EPS = 1e-5
F32, BF16, U32 = jnp.float32, jnp.bfloat16, jnp.uint32

NN = (((1,), (0,)), ((), ()))


def _dot(a, b, dims=NN):
    return lax.dot_general(a, b, dims, preferred_element_type=F32)


def _ln(x):
    m = jnp.mean(x, axis=-1, keepdims=True)
    c = x - m
    v = jnp.mean(c * c, axis=-1, keepdims=True)
    return c * lax.rsqrt(v + EPS)


def _unpack(w):
    lo = pltpu.unpack_elementwise(w, index=0, packed_dtype=BF16, unpacked_dtype=F32)
    hi = pltpu.unpack_elementwise(w, index=1, packed_dtype=BF16, unpacked_dtype=F32)
    return lo, hi


def _pk(x):
    return pltpu.bitcast(x.astype(BF16), U32)


def _bf(w):
    return pltpu.bitcast(w, BF16)


def make(R=256, LNC=32, LNB=32, NL=2, WOS=5, WAITS=(0, 1, 2, 3, 4, 5, 6, 7), AHEAD=9, AF=(0, 1), DEFER=1,
         SCOPES=False, W32=1, UNS=1, HALO=0, EX2=0, QKF=0, KO=(0, 1, 2), WC=0, ONLY=None, LNP=0):
    NB = S // R
    assert R == 256
    GR = 128
    NG = D // GR
    NH = DH // 8
    GP = GR // 2
    XN0 = S + R
    QX0 = 3 * D
    NQ = D // 128

    def scoped(name, fn):
        if SCOPES:
            with jax.named_scope(name):
                fn()
        else:
            fn()

    def kernel(x_hbm, wqkv_hbm, wo_hbm, w1_hbm, b1_hbm, w2_hbm, b2_hbm, out_hbm,
               xin, wqkv, wo, wq32, wo32, w1, w2, bb1, bb2, xa, xb, qkv, qkv0, kprev, vprev, o, h, ostage, b1_ref, b2_ref,
               sem_x, sem_qkv, sem_w, sem_o, sem_c, sem_f):
        cp_q = [[pltpu.make_async_copy(wqkv_hbm.at[:, pl.ds(p * D + g * GR, GR)],
                                       wqkv.at[:, pl.ds(p * D + g * GR, GR)],
                                       sem_qkv.at[g * 3 + p]) for p in range(3)] for g in range(NG)]

        def rows(r, n):
            return pl.ds(r if isinstance(r, int) else pl.multiple_of(r, n), n)

        def blk(i):
            return rows(i * R, R)

        def cp_x(i):
            return pltpu.make_async_copy(x_hbm.at[blk(i)], xin.at[blk(i)], sem_x.at[i])

        def cp_o(i):
            return pltpu.make_async_copy(ostage.at[blk(i)], out_hbm.at[blk(i)], sem_o.at[i])

        cp_ba = pltpu.make_async_copy(xb.at[blk(0)], xa.at[blk(NB)], sem_c.at[0])
        cp_ab = pltpu.make_async_copy(xa.at[blk(0)], xb.at[blk(NB)], sem_c.at[1])

        k1 = WOS * GR
        cp_wo1 = pltpu.make_async_copy(wo_hbm.at[:k1], wo.at[:k1], sem_w.at[0])
        cp_wo2 = pltpu.make_async_copy(wo_hbm.at[k1:], wo.at[k1:], sem_w.at[3])
        cp_b1 = pltpu.make_async_copy(b1_hbm, b1_ref, sem_w.at[4])
        cp_b2 = pltpu.make_async_copy(b2_hbm, b2_ref, sem_w.at[5])
        cp_w1 = pltpu.make_async_copy(w1_hbm, w1, sem_w.at[1])
        cp_w2 = pltpu.make_async_copy(w2_hbm, w2, sem_w.at[2])

        queue = [[cp_x(0)]] + [cp_q[0] + [cp_b1, cp_b2]] + cp_q[1:] + [[cp_wo1], [cp_x(1), cp_wo2]]
        issued = [0]

        def issue(n):
            while issued[0] < min(n, len(queue)):
                for c in queue[issued[0]]:
                    c.start()
                issued[0] += 1

        issue(1)
        pl.semaphore_signal(sem_f)
        pl.semaphore_wait(sem_f)
        issue(2)


        def get_xn():
            return pltpu.bitcast(xb[pl.ds(XN0, R // 2), :], BF16)

        def load_x(src_ref, i, off, n, from_input):
            sl = rows(i * R + off, n)
            if from_input is False:
                return src_ref[sl, :]
            if from_input is True:
                return xin[sl, :].astype(F32)
            si = rows(jnp.minimum(i, NB - 1) * R + off, n)
            return jnp.where(from_input, xin[si, :].astype(F32), src_ref[sl, :])

        def layernorm(src_ref, i, from_input=False, zero=0):
            for c in range(R // LNB):
                y = _ln(load_x(src_ref, i, c * LNB, LNB, from_input))
                xb[rows(zero + XN0 + c * LNB // 2, LNB // 2), :] = pltpu.bitcast(y.astype(BF16), F32)

        def layernorm_staged(i, zero, from_input):
            for c in range(R // LNC):
                y = _pk(_ln(load_x(xa, i, c * LNC, LNC, from_input)))
                for k in range(NQ):
                    qkv[rows(zero + QX0 + k * (R // 2) + c * LNC // 2, LNC // 2), :] = y[:, k * 128:(k + 1) * 128]

        def unstage():
            for k in range(NQ):
                xb[pl.ds(XN0, R // 2), pl.ds(k * 128, 128)] = pltpu.bitcast(
                    qkv[pl.ds(QX0 + k * (R // 2), R // 2), :], F32)

        lane = lax.broadcasted_iota(jnp.int32, (8, 128), 1)
        sub = lax.broadcasted_iota(jnp.int32, (8, 128), 0)
        m_even = (sub & 2) == 0
        m_odd = ((sub + 7) & 2) == 0
        m_par = (sub & 1) == 0

        def attention(g, first):
            base = g * 3 * GR

            def shifted(part, prev_ref, d):
                cur = qkv[pl.ds(base + part * GR + d * 8, 8), :]
                out = [_unpack(cur)]
                if first is True or part == 2:
                    b = jnp.broadcast_to(out[0][0][:, 0:1], (8, 128))
                    prev = pltpu.pack_elementwise([b, b], packed_dtype=BF16)
                if first is not True:
                    old = prev_ref[pl.ds(g * GR + d * 8, 8), :]
                    prev = jnp.where(first, prev, old) if part == 2 else old
                for w in range(1, WIN):
                    out.append(_unpack(pltpu.roll(jnp.where(lane >= 128 - w, prev, cur), w, 1)))
                return out

            def probs(hp):
                half = []
                for hd in (2 * hp, 2 * hp + 1):
                    acc = [[None, None] for _ in range(WIN)]
                    for d in range(hd * NH, (hd + 1) * NH):
                        q = _unpack(qkv[pl.ds(base + d * 8, 8), :])
                        ks = shifted(1, kprev, d)
                        for w in range(WIN):
                            for k in range(2):
                                pr = q[k] * ks[w][k]
                                acc[w][k] = pr if acc[w][k] is None else acc[w][k] + pr
                    m = m_odd if hd % 2 else m_even
                    half.append([jnp.where(m, a, b) + pltpu.roll(jnp.where(m, b, a), 6, 0) for a, b in acc])
                lg = []
                for u, v in zip(*half):
                    z = jnp.where(m_par, u, v) + pltpu.roll(jnp.where(m_par, v, u), 7, 0)
                    lg.append((z + pltpu.roll(z, 4, 0)) * (DH ** -0.5))
                lg = [lg[0]] + [jnp.where(jnp.logical_and(first, lane < w), -1e9, lg[w]) for w in range(1, WIN)]
                mx = functools.reduce(jnp.maximum, lg)
                e = [jnp.exp(a - mx) for a in lg]
                inv = 1.0 / functools.reduce(jnp.add, e)
                return [a * inv for a in e]

            def values(hp, p):
                outs = []
                for hd in (2 * hp, 2 * hp + 1):
                    ph = [[jnp.broadcast_to(a[hd % 2 + 2 * k:hd % 2 + 2 * k + 1, :], (8, 128)) for k in range(2)]
                          for a in p]
                    for d in range(hd * NH, (hd + 1) * NH):
                        vs = shifted(2, vprev, d)
                        os_ = []
                        for k in range(2):
                            if EX2:
                                t = [ph[w][k] * vs[w][k] for w in range(WIN)]
                                acc_o = ((t[0] + t[1]) + (t[2] + t[3])) + ((t[4] + t[5]) + (t[6] + t[7]))
                            else:
                                acc_o = ph[0][k] * vs[0][k]
                                for w in range(1, WIN):
                                    acc_o = acc_o + ph[w][k] * vs[w][k]
                            os_.append(acc_o)
                        outs.append(pltpu.pack_elementwise(os_, packed_dtype=BF16))
                return outs

            if QKF:
                ps = [probs(0), probs(1)]
                outs = values(0, ps[0]) + values(1, ps[1])
            else:
                outs = values(0, probs(0)) + values(1, probs(1))
            o[:, pl.ds(g * GR, GR)] = jnp.concatenate(outs, axis=0).T
            if HALO == 0:
                save_halo(g)

        def save_halo(g):
            kprev[pl.ds(g * GR, GR), :] = qkv[pl.ds((g * 3 + 1) * GR, GR), :]
            vprev[pl.ds(g * GR, GR), :] = qkv[pl.ds((g * 3 + 2) * GR, GR), :]

        def fold(a):
            u = jnp.where(m_even, a[0], a[2]) + pltpu.roll(jnp.where(m_even, a[2], a[0]), 6, 0)
            v = jnp.where(m_odd, a[1], a[3]) + pltpu.roll(jnp.where(m_odd, a[3], a[1]), 6, 0)
            z = jnp.where(m_par, u, v) + pltpu.roll(jnp.where(m_par, v, u), 7, 0)
            return z + pltpu.roll(z, 4, 0)

        def attention_first(g):
            base = g * 3 * GP
            for t in range(R // 128):
                cols = pl.ds(t * 128, 128)

                def shifted(part, d):
                    rs = pl.ds(base + part * GP + d * 8, 8)
                    cur = qkv0[rs, cols]
                    if t == 0:
                        prev = jnp.broadcast_to(cur[:, 0:1], (8, 128))
                    else:
                        prev = qkv0[rs, pl.ds((t - 1) * 128, 128)]
                    out = [_unpack(cur)]
                    for w in range(1, WIN):
                        sh = w * DIL
                        out.append(_unpack(pltpu.roll(jnp.where(lane >= 128 - sh, prev, cur), sh, 1)))
                    return out

                acc = [[None] * 4 for _ in range(WIN)]
                for d in range(GP // 8):
                    hd = d // 2
                    q0, q1 = _unpack(qkv0[pl.ds(base + d * 8, 8), cols])
                    ks = shifted(1, d)
                    for w in range(WIN):
                        pr = q0 * ks[w][0] + q1 * ks[w][1]
                        acc[w][hd] = pr if acc[w][hd] is None else acc[w][hd] + pr
                lg = [fold(a) * (DH ** -0.5) for a in acc]
                if t == 0:
                    lg = [lg[0]] + [jnp.where(lane < w * DIL, -1e9, lg[w])
                                    for w in range(1, WIN)]
                m = functools.reduce(jnp.maximum, lg)
                e = [jnp.exp(a - m) for a in lg]
                inv = 1.0 / functools.reduce(jnp.add, e)
                p = [a * inv for a in e]
                outs = []
                for d in range(GP // 8):
                    hd = d // 2
                    if d % 2 == 0:
                        ph = [jnp.broadcast_to(a[hd:hd + 1, :], (8, 128)) for a in p]
                    vs = shifted(2, d)
                    os_ = []
                    for k in range(2):
                        acc_o = ph[0] * vs[0][k]
                        for w in range(1, WIN):
                            acc_o = acc_o + ph[w] * vs[w][k]
                        os_.append(acc_o)
                    outs.append(_bf(pltpu.pack_elementwise(os_, packed_dtype=BF16)))
                oT = jnp.concatenate(outs, axis=0)
                o[pl.ds(t * 64, 64), pl.ds(g * GR, GR)] = pltpu.bitcast(oT.T, U32)

        def attn_unit(i, l, peeled=False):
            first = True if peeled else i == 0
            waited = [0]
            pending = []

            def flush():
                while pending:
                    g, p = pending.pop(0)
                    qkv0[pl.ds((g * 3 + p) * GP, GP), :] = pltpu.bitcast(_bf(vprev[pl.ds(g * GR, GR), :]).T, U32)

            def need(g):
                if peeled and waited[0] <= g < NG:
                    nxt = min([w for w in WAITS if w > g] + [NG])
                    issue(nxt + 1)
                    for gg in range(waited[0], nxt):
                        scoped(f"wq{gg}", lambda: [c.wait() for c in cp_q[gg]] and None)
                    issue(nxt + 1 + AHEAD)
                    if waited[0] == 0:
                        cp_b1.wait()
                        cp_b2.wait()
                        bb1[...] = jnp.broadcast_to(b1_ref[...].astype(F32).reshape(1, F), (8, F))
                        bb2[...] = jnp.broadcast_to(b2_ref[...].astype(F32).reshape(1, D), (8, D))
                    waited[0] = nxt
                    flush()

            def proj(g):
                need(g)
                for n, p in enumerate((0, 1, 2) if peeled else KO):
                    if g == 0 and n == LNP and not peeled:
                        layernorm_staged(i + 1, i >> 8, jnp.logical_and(l == 0, i + 1 < NB))
                    cs = pl.ds(p * D + g * GR, GR)
                    if W32 and not peeled:
                        wv = _bf(wq32[:, cs])
                    else:
                        wv = wqkv[:, cs]
                        if W32:
                            wq32[:, cs] = pltpu.bitcast(wv, U32)
                    y = _pk(_dot(get_xn(), wv))
                    if not peeled:
                        qkv[pl.ds((g * 3 + p) * GR, GR), :] = y.T
                        continue
                    if p:
                        (kprev, vprev)[p - 1][pl.ds(g * GR, GR), :] = y
                    if p == 2 and (g + 1 in WAITS or g + 1 == NG):
                        pending.append((g, p))
                    else:
                        qkv0[pl.ds((g * 3 + p) * GP, GP), :] = pltpu.bitcast(_bf(y).T, U32)

            def attend(g):
                if peeled:
                    attention_first(g)
                else:
                    attention(g, first)

            proj(0)
            for g in range(NG - 1):
                if AF[int(peeled)]:
                    need(g + 1)
                    attend(g)
                    proj(g + 1)
                else:
                    proj(g + 1)
                    attend(g)
            if peeled:
                issue(len(queue))
                scoped("wwo1", cp_wo1.wait)
                for j in range(2, NB):
                    cp_x(j).start()
                flush()
            if UNS == 0 and not peeled:
                unstage()

            def get_wo(a, b, cs):
                if W32 == 2 and not peeled:
                    return _bf(wo32[a // 2:b // 2, cs])
                wv = wo[a:b, cs]
                if W32 == 2:
                    wo32[a // 2:b // 2, cs] = pltpu.bitcast(wv, U32)
                return wv

            y = _dot(_bf(o[:, :k1]), get_wo(0, k1, slice(None)))
            xb[blk(i), :] = load_x(xa, i, 0, R, True if peeled else l == 0) + y
            attend(NG - 1)
            if peeled:
                scoped("wx1", cp_x(1).wait)
                scoped("wwo2", cp_wo2.wait)
                cp_w1.start()
                cp_w2.start()
                layernorm(xa, 1, True, pl.program_id(0))
                for g in range(NG):
                    for ref in (kprev, vprev):
                        ref[pl.ds(g * GR, GR), :] = ref[pl.ds(g * GR, GR), :].T
            elif UNS == 1:
                unstage()
            if HALO and not peeled:
                for g in range(NG):
                    save_halo(g)
            nc = D // WC if WC else D
            for c in range(0, D, nc):
                cs = pl.ds(c, nc)
                xb[blk(i), cs] = xb[blk(i), cs] + _dot(_bf(o[:, k1:]), get_wo(k1, D, cs))

        def ffn_unit(i):
            hh = _dot(get_xn(), w1[...]) + bb1[0:1, :]
            rr = jnp.where(hh > 0, hh, 0.0)
            h[...] = _pk(rr * rr)
            layernorm(xb, i + 1)
            x2 = xb[blk(i), :] + (_dot(_bf(h[...]), w2[...]) + bb2[0:1, :])
            xa[blk(i), :] = x2
            ostage[blk(i), :] = x2.astype(BF16)

        scoped("wait_x0", lambda: cp_x(0).wait())
        issue(1 + AHEAD)
        layernorm(xa, 0, True)
        if ONLY in (None, "P"):
            scoped("attn_first", lambda: attn_unit(0, 0, True))

        def layer(l, carry):
            def _a(i, c):
                @pl.when(jnp.logical_and(l == 0, i + 1 < NB))
                def _():
                    cp_x(i + 1).wait()

                @pl.when(i == 1)
                def _():
                    cp_ba.start()

                @pl.when(i == NB - 1)
                def _():
                    cp_ba.wait()

                scoped("attn_unit", lambda: attn_unit(i, l))
                return c
            if ONLY in (None, "A"):
                lax.fori_loop(jnp.where(l == 0, 1, 0), NB, _a, 0)

            @pl.when(l == 0)
            def _():
                cp_w1.wait()
                cp_w2.wait()

            def _b(i, c):
                @pl.when(i == 1)
                def _():
                    cp_ab.start()

                @pl.when(i == NB - 1)
                def _():
                    cp_ab.wait()

                scoped("ffn_unit", lambda: ffn_unit(i))

                @pl.when(l == NL - 1)
                def _():
                    cp_o(i).start()
                return c
            if ONLY in (None, "B"):
                lax.fori_loop(0, NB, _b, 0)
            return carry

        lax.fori_loop(0, NL, layer, 0)
        for i in range(NB):
            cp_o(i).wait()

    def run(A_x, A_wqkv, A_wo, B_x, B_w1, B_b1, B_w2, B_b2):
        del B_x
        hbm = pl.BlockSpec(memory_space=pl.ANY)
        out = pl.pallas_call(
            kernel,
            out_shape=jax.ShapeDtypeStruct((S, D), BF16),
            grid=(1,),
            in_specs=[hbm] * 7,
            out_specs=hbm,
            scratch_shapes=[
                pltpu.VMEM((S, D), BF16),
                pltpu.VMEM((D, 3 * D), BF16),
                pltpu.VMEM((D, D), BF16),
                pltpu.VMEM((D // 2, 3 * D), U32),
                pltpu.VMEM((D // 2, D), U32),
                pltpu.VMEM((D, F), BF16),
                pltpu.VMEM((F, D), BF16),
                pltpu.VMEM((8, F), F32),
                pltpu.VMEM((8, D), F32),
                pltpu.VMEM((S + R, D), F32),
                pltpu.VMEM((S + R + R // 2, D), F32),
                pltpu.VMEM((4 * D, 128), U32),
                pltpu.VMEM((3 * D // 2, R), U32),
                pltpu.VMEM((D, 128), U32),
                pltpu.VMEM((D, 128), U32),
                pltpu.VMEM((R // 2, D), U32),
                pltpu.VMEM((R // 2, F), U32),
                pltpu.VMEM((S, D), BF16),
                pltpu.VMEM((F,), BF16),
                pltpu.VMEM((D,), BF16),
                pltpu.SemaphoreType.DMA((NB,)),
                pltpu.SemaphoreType.DMA((3 * NG,)),
                pltpu.SemaphoreType.DMA((6,)),
                pltpu.SemaphoreType.DMA((NB,)),
                pltpu.SemaphoreType.DMA((2,)),
                pltpu.SemaphoreType.REGULAR,
            ],
            compiler_params=pltpu.CompilerParams(vmem_limit_bytes=110 * 1024 * 1024),
        )(A_x.reshape(S, D), A_wqkv, A_wo, B_w1, B_b1, B_w2, B_b2)
        return out.reshape(1, S, D)

    return run


@jax.jit
def pallas_interleave_layers__sliding_local_dilated__dense_activation_squared_relu__prompt_kernel(A_x, A_wqkv, A_wo, B_x, B_w1, B_b1, B_w2, B_b2):
    return make()(A_x, A_wqkv, A_wo, B_x, B_w1, B_b1, B_w2, B_b2)
```

```python
import functools
import numpy as np
import jax
import jax.numpy as jnp
from jax import lax
import jax.experimental.pallas as pl
import jax.experimental.pallas.tpu as pltpu

S, D, F, H, DH = 2048, 1024, 3584, 32, 32
WIN, DIL = 8, 2
EPS = 1e-5
F32, BF16, U32 = jnp.float32, jnp.bfloat16, jnp.uint32

NN = (((1,), (0,)), ((), ()))


def _dot(a, b, dims=NN):
    return lax.dot_general(a, b, dims, preferred_element_type=F32)


def _ln(x):
    m = jnp.mean(x, axis=-1, keepdims=True)
    c = x - m
    v = jnp.mean(c * c, axis=-1, keepdims=True)
    return c * lax.rsqrt(v + EPS)


def _unpack(w):
    lo = pltpu.unpack_elementwise(w, index=0, packed_dtype=BF16, unpacked_dtype=F32)
    hi = pltpu.unpack_elementwise(w, index=1, packed_dtype=BF16, unpacked_dtype=F32)
    return lo, hi


def _pk(x):
    return pltpu.bitcast(x.astype(BF16), U32)


def _bf(w):
    return pltpu.bitcast(w, BF16)


def make(R=256, LNC=32, LNB=32, NL=2, WOS=5, WAITS=(0, 1, 2, 3, 4, 5, 6), AHEAD=9, AF=(0, 1), DEFER=1,
         SCOPES=False, OC=4, CARRY=0, XV=0, W32=1, UNS=1, HALO=0, EX2=0, QKF=0, KO=(0, 1, 2), WC=0, ONLY=None, LNP=0):
    NB = S // R
    assert R == 256
    GR = 128
    NG = D // GR
    NH = DH // 8
    GP = GR // 2
    XN0 = S + R
    QX0 = 3 * D
    NQ = D // 128

    def scoped(name, fn):
        if SCOPES:
            with jax.named_scope(name):
                fn()
        else:
            fn()

    def kernel(x_hbm, wqkv_hbm, wo_hbm, w1_hbm, b1_hbm, w2_hbm, b2_hbm, out_hbm,
               xin, wqkv, wo, wq32, wo32, w1, w2, bb1, bb2, xa, xb, qkv, qkv0, kprev, vprev, o, h, ostage, b1_ref, b2_ref,
               sem_x, sem_qkv, sem_w, sem_o, sem_c, sem_f):
        cp_q = [[pltpu.make_async_copy(wqkv_hbm.at[:, pl.ds(p * D + g * GR, GR)],
                                       wqkv.at[:, pl.ds(p * D + g * GR, GR)],
                                       sem_qkv.at[g * 3 + p]) for p in range(3)] for g in range(NG)]

        def rows(r, n):
            return pl.ds(r if isinstance(r, int) else pl.multiple_of(r, n), n)

        def blk(i):
            return rows(i * R, R)

        def cp_x(i):
            return pltpu.make_async_copy(x_hbm.at[blk(i)], xin.at[blk(i)], sem_x.at[i])

        def cp_o(i, c):
            cs = pl.ds(c * (D // OC), D // OC)
            return pltpu.make_async_copy(ostage.at[blk(i), cs], out_hbm.at[blk(i), cs], sem_o.at[i, c])

        cp_ba = pltpu.make_async_copy(xb.at[blk(0)], xa.at[blk(NB)], sem_c.at[0])
        cp_ab = pltpu.make_async_copy(xa.at[blk(0)], xb.at[blk(NB)], sem_c.at[1])

        k1 = WOS * GR
        cp_wo1 = pltpu.make_async_copy(wo_hbm.at[:k1], wo.at[:k1], sem_w.at[0])
        cp_wo2 = pltpu.make_async_copy(wo_hbm.at[k1:], wo.at[k1:], sem_w.at[3])
        cp_b1 = pltpu.make_async_copy(b1_hbm, b1_ref, sem_w.at[4])
        cp_b2 = pltpu.make_async_copy(b2_hbm, b2_ref, sem_w.at[5])
        cp_w1 = pltpu.make_async_copy(w1_hbm, w1, sem_w.at[1])
        cp_w2 = pltpu.make_async_copy(w2_hbm, w2, sem_w.at[2])

        queue = [[cp_x(0)]] + [cp_q[0] + [cp_b1, cp_b2]] + cp_q[1:] + [[cp_wo1], [cp_x(1), cp_wo2]]
        issued = [0]

        def issue(n):
            while issued[0] < min(n, len(queue)):
                for c in queue[issued[0]]:
                    c.start()
                issued[0] += 1

        issue(1)
        pl.semaphore_signal(sem_f)
        pl.semaphore_wait(sem_f)
        issue(2)


        def get_xn():
            return pltpu.bitcast(xb[pl.ds(XN0, R // 2), :], BF16)

        def load_x(src_ref, i, off, n, from_input):
            sl = rows(i * R + off, n)
            if from_input is False:
                return src_ref[sl, :]
            if from_input is True:
                return xin[sl, :].astype(F32)
            si = rows(jnp.minimum(i, NB - 1) * R + off, n)
            return jnp.where(from_input, xin[si, :].astype(F32), src_ref[sl, :])

        def layernorm(src_ref, i, from_input=False, zero=0):
            for c in range(R // LNB):
                y = _ln(load_x(src_ref, i, c * LNB, LNB, from_input))
                xb[rows(zero + XN0 + c * LNB // 2, LNB // 2), :] = pltpu.bitcast(y.astype(BF16), F32)

        def layernorm_staged(i, zero, from_input):
            for c in range(R // LNC):
                y = _pk(_ln(load_x(xa, i, c * LNC, LNC, from_input)))
                for k in range(NQ):
                    qkv[rows(zero + QX0 + k * (R // 2) + c * LNC // 2, LNC // 2), :] = y[:, k * 128:(k + 1) * 128]

        def unstage():
            for k in range(NQ):
                xb[pl.ds(XN0, R // 2), pl.ds(k * 128, 128)] = pltpu.bitcast(
                    qkv[pl.ds(QX0 + k * (R // 2), R // 2), :], F32)

        lane = lax.broadcasted_iota(jnp.int32, (8, 128), 1)
        sub = lax.broadcasted_iota(jnp.int32, (8, 128), 0)
        m_even = (sub & 2) == 0
        m_odd = ((sub + 7) & 2) == 0
        m_par = (sub & 1) == 0

        def attention(g, first):
            base = g * 3 * GR

            def shifted(part, prev_ref, d):
                cur = qkv[pl.ds(base + part * GR + d * 8, 8), :]
                out = [_unpack(cur)]
                if first is True or part == 2:
                    b = jnp.broadcast_to(out[0][0][:, 0:1], (8, 128))
                    prev = pltpu.pack_elementwise([b, b], packed_dtype=BF16)
                if first is not True:
                    old = prev_ref[pl.ds(g * GR + d * 8, 8), :]
                    prev = jnp.where(first, prev, old) if part == 2 else old
                for w in range(1, WIN):
                    out.append(_unpack(pltpu.roll(jnp.where(lane >= 128 - w, prev, cur), w, 1)))
                return out

            def probs(hp):
                half = []
                for hd in (2 * hp, 2 * hp + 1):
                    acc = [[None, None] for _ in range(WIN)]
                    for d in range(hd * NH, (hd + 1) * NH):
                        q = _unpack(qkv[pl.ds(base + d * 8, 8), :])
                        ks = shifted(1, kprev, d)
                        for w in range(WIN):
                            for k in range(2):
                                pr = q[k] * ks[w][k]
                                acc[w][k] = pr if acc[w][k] is None else acc[w][k] + pr
                    m = m_odd if hd % 2 else m_even
                    half.append([jnp.where(m, a, b) + pltpu.roll(jnp.where(m, b, a), 6, 0) for a, b in acc])
                lg = []
                for u, v in zip(*half):
                    z = jnp.where(m_par, u, v) + pltpu.roll(jnp.where(m_par, v, u), 7, 0)
                    lg.append((z + pltpu.roll(z, 4, 0)) * (DH ** -0.5))
                lg = [lg[0]] + [jnp.where(jnp.logical_and(first, lane < w), -1e9, lg[w]) for w in range(1, WIN)]
                mx = functools.reduce(jnp.maximum, lg)
                e = [jnp.exp(a - mx) for a in lg]
                inv = 1.0 / functools.reduce(jnp.add, e)
                return [a * inv for a in e]

            def values(hp, p):
                outs = []
                for hd in (2 * hp, 2 * hp + 1):
                    ph = [[jnp.broadcast_to(a[hd % 2 + 2 * k:hd % 2 + 2 * k + 1, :], (8, 128)) for k in range(2)]
                          for a in p]
                    for d in range(hd * NH, (hd + 1) * NH):
                        vs = shifted(2, vprev, d)
                        os_ = []
                        for k in range(2):
                            if EX2:
                                t = [ph[w][k] * vs[w][k] for w in range(WIN)]
                                acc_o = ((t[0] + t[1]) + (t[2] + t[3])) + ((t[4] + t[5]) + (t[6] + t[7]))
                            else:
                                acc_o = ph[0][k] * vs[0][k]
                                for w in range(1, WIN):
                                    acc_o = acc_o + ph[w][k] * vs[w][k]
                            os_.append(acc_o)
                        outs.append(pltpu.pack_elementwise(os_, packed_dtype=BF16))
                return outs

            if QKF:
                ps = [probs(0), probs(1)]
                outs = values(0, ps[0]) + values(1, ps[1])
            else:
                outs = values(0, probs(0)) + values(1, probs(1))
            o[:, pl.ds(g * GR, GR)] = jnp.concatenate(outs, axis=0).T
            if HALO == 0:
                save_halo(g)

        def save_halo(g):
            kprev[pl.ds(g * GR, GR), :] = qkv[pl.ds((g * 3 + 1) * GR, GR), :]
            vprev[pl.ds(g * GR, GR), :] = qkv[pl.ds((g * 3 + 2) * GR, GR), :]

        def fold(a):
            u = jnp.where(m_even, a[0], a[2]) + pltpu.roll(jnp.where(m_even, a[2], a[0]), 6, 0)
            v = jnp.where(m_odd, a[1], a[3]) + pltpu.roll(jnp.where(m_odd, a[3], a[1]), 6, 0)
            z = jnp.where(m_par, u, v) + pltpu.roll(jnp.where(m_par, v, u), 7, 0)
            return z + pltpu.roll(z, 4, 0)

        def attention_first(g):
            base = g * 3 * GP
            for t in range(R // 128):
                cols = pl.ds(t * 128, 128)

                def shifted(part, d):
                    rs = pl.ds(base + part * GP + d * 8, 8)
                    cur = qkv0[rs, cols]
                    if t == 0:
                        prev = jnp.broadcast_to(cur[:, 0:1], (8, 128))
                    else:
                        prev = qkv0[rs, pl.ds((t - 1) * 128, 128)]
                    out = [_unpack(cur)]
                    for w in range(1, WIN):
                        sh = w * DIL
                        out.append(_unpack(pltpu.roll(jnp.where(lane >= 128 - sh, prev, cur), sh, 1)))
                    return out

                acc = [[None] * 4 for _ in range(WIN)]
                for d in range(GP // 8):
                    hd = d // 2
                    q0, q1 = _unpack(qkv0[pl.ds(base + d * 8, 8), cols])
                    ks = shifted(1, d)
                    for w in range(WIN):
                        pr = q0 * ks[w][0] + q1 * ks[w][1]
                        acc[w][hd] = pr if acc[w][hd] is None else acc[w][hd] + pr
                lg = [fold(a) * (DH ** -0.5) for a in acc]
                if t == 0:
                    lg = [lg[0]] + [jnp.where(lane < w * DIL, -1e9, lg[w])
                                    for w in range(1, WIN)]
                m = functools.reduce(jnp.maximum, lg)
                e = [jnp.exp(a - m) for a in lg]
                inv = 1.0 / functools.reduce(jnp.add, e)
                p = [a * inv for a in e]
                outs = []
                for d in range(GP // 8):
                    hd = d // 2
                    if d % 2 == 0:
                        ph = [jnp.broadcast_to(a[hd:hd + 1, :], (8, 128)) for a in p]
                    vs = shifted(2, d)
                    os_ = []
                    for k in range(2):
                        acc_o = ph[0] * vs[0][k]
                        for w in range(1, WIN):
                            acc_o = acc_o + ph[w] * vs[w][k]
                        os_.append(acc_o)
                    outs.append(_bf(pltpu.pack_elementwise(os_, packed_dtype=BF16)))
                oT = jnp.concatenate(outs, axis=0)
                o[pl.ds(t * 64, 64), pl.ds(g * GR, GR)] = pltpu.bitcast(oT.T, U32)

        def attn_unit(i, l, peeled=False):
            first = True if peeled else i == 0
            waited = [0]
            xn0 = get_xn() if peeled and XV else None
            pending = []

            def flush():
                while pending:
                    g, p, y = pending.pop(0)
                    if y is None:
                        y = vprev[pl.ds(g * GR, GR), :]
                    elif p:
                        (kprev, vprev)[p - 1][pl.ds(g * GR, GR), :] = y
                    qkv0[pl.ds((g * 3 + p) * GP, GP), :] = pltpu.bitcast(_bf(y).T, U32)

            def need(g):
                if peeled and waited[0] <= g < NG:
                    nxt = min([w for w in WAITS if w > g] + [NG])
                    issue(nxt + 1)
                    for gg in range(waited[0], nxt):
                        scoped(f"wq{gg}", lambda: [c.wait() for c in cp_q[gg]] and None)
                    issue(nxt + 1 + AHEAD)
                    if waited[0] == 0:
                        cp_b1.wait()
                        cp_b2.wait()
                        bb1[...] = jnp.broadcast_to(b1_ref[...].astype(F32).reshape(1, F), (8, F))
                        bb2[...] = jnp.broadcast_to(b2_ref[...].astype(F32).reshape(1, D), (8, D))
                    waited[0] = nxt
                    flush()

            def proj(g, after=None):
                need(g)
                if after:
                    after()
                for n, p in enumerate((0, 1, 2) if peeled else KO):
                    if g == 0 and n == LNP and not peeled:
                        layernorm_staged(i + 1, i >> 8, jnp.logical_and(l == 0, i + 1 < NB))
                    cs = pl.ds(p * D + g * GR, GR)
                    if W32 and not peeled:
                        wv = _bf(wq32[:, cs])
                    else:
                        wv = wqkv[:, cs]
                        if W32:
                            wq32[:, cs] = pltpu.bitcast(wv, U32)
                    y = _pk(_dot(xn0 if peeled and XV else get_xn(), wv))
                    if not peeled:
                        qkv[pl.ds((g * 3 + p) * GR, GR), :] = y.T
                        continue
                    if p >= 3 - CARRY:
                        pending.append((g, p, y))
                        continue
                    if p:
                        (kprev, vprev)[p - 1][pl.ds(g * GR, GR), :] = y
                    if p == 2 and (g + 1 in WAITS or g + 1 == NG):
                        pending.append((g, p, None))
                    else:
                        qkv0[pl.ds((g * 3 + p) * GP, GP), :] = pltpu.bitcast(_bf(y).T, U32)

            def attend(g):
                if peeled:
                    attention_first(g)
                else:
                    attention(g, first)

            proj(0)
            for g in range(NG - 1):
                if peeled and AF[1] == 2:
                    need(g + 1)
                    proj(g + 1)
                    attend(g)
                elif AF[int(peeled)]:
                    need(g + 1)
                    attend(g)
                    proj(g + 1)
                else:
                    proj(g + 1)
                    attend(g)
            if peeled:
                issue(len(queue))
                scoped("wwo1", cp_wo1.wait)
                for j in range(2, NB):
                    cp_x(j).start()
                flush()
            if UNS == 0 and not peeled:
                unstage()

            def get_wo(a, b, cs):
                if W32 == 2 and not peeled:
                    return _bf(wo32[a // 2:b // 2, cs])
                wv = wo[a:b, cs]
                if W32 == 2:
                    wo32[a // 2:b // 2, cs] = pltpu.bitcast(wv, U32)
                return wv

            y = _dot(_bf(o[:, :k1]), get_wo(0, k1, slice(None)))
            xb[blk(i), :] = load_x(xa, i, 0, R, True if peeled else l == 0) + y
            attend(NG - 1)
            if peeled:
                scoped("wx1", cp_x(1).wait)
                scoped("wwo2", cp_wo2.wait)
                cp_w1.start()
                cp_w2.start()
                layernorm(xa, 1, True, pl.program_id(0))
                for g in range(NG):
                    for ref in (kprev, vprev):
                        ref[pl.ds(g * GR, GR), :] = ref[pl.ds(g * GR, GR), :].T
            elif UNS == 1:
                unstage()
            if HALO and not peeled:
                for g in range(NG):
                    save_halo(g)
            nc = D // WC if WC else D
            for c in range(0, D, nc):
                cs = pl.ds(c, nc)
                xb[blk(i), cs] = xb[blk(i), cs] + _dot(_bf(o[:, k1:]), get_wo(k1, D, cs))

        def ffn_unit(i, l):
            hh = _dot(get_xn(), w1[...]) + bb1[0:1, :]
            rr = jnp.where(hh > 0, hh, 0.0)
            h[...] = _pk(rr * rr)
            layernorm(xb, i + 1)
            for c in range(OC):
                cs = pl.ds(c * (D // OC), D // OC)
                x2 = xb[blk(i), cs] + (_dot(_bf(h[...]), w2[:, cs]) + bb2[0:1, cs])
                xa[blk(i), cs] = x2
                ostage[blk(i), cs] = x2.astype(BF16)

                @pl.when(l == NL - 1)
                def _():
                    cp_o(i, c).start()

        scoped("wait_x0", lambda: cp_x(0).wait())
        issue(1 + AHEAD)
        layernorm(xa, 0, True)
        if ONLY in (None, "P"):
            scoped("attn_first", lambda: attn_unit(0, 0, True))

        def layer(l, carry):
            def _a(i, c):
                @pl.when(jnp.logical_and(l == 0, i + 1 < NB))
                def _():
                    cp_x(i + 1).wait()

                @pl.when(i == 1)
                def _():
                    cp_ba.start()

                @pl.when(i == NB - 1)
                def _():
                    cp_ba.wait()

                scoped("attn_unit", lambda: attn_unit(i, l))
                return c
            if ONLY in (None, "A"):
                lax.fori_loop(jnp.where(l == 0, 1, 0), NB, _a, 0)

            @pl.when(l == 0)
            def _():
                cp_w1.wait()
                cp_w2.wait()

            def _b(i, c):
                @pl.when(i == 1)
                def _():
                    cp_ab.start()

                @pl.when(i == NB - 1)
                def _():
                    cp_ab.wait()

                scoped("ffn_unit", lambda: ffn_unit(i, l))
                return c
            if ONLY in (None, "B"):
                lax.fori_loop(0, NB, _b, 0)
            return carry

        lax.fori_loop(0, NL, layer, 0)
        for i in range(NB):
            for c in range(OC):
                cp_o(i, c).wait()

    def run(A_x, A_wqkv, A_wo, B_x, B_w1, B_b1, B_w2, B_b2):
        del B_x
        hbm = pl.BlockSpec(memory_space=pl.ANY)
        out = pl.pallas_call(
            kernel,
            out_shape=jax.ShapeDtypeStruct((S, D), BF16),
            grid=(1,),
            in_specs=[hbm] * 7,
            out_specs=hbm,
            scratch_shapes=[
                pltpu.VMEM((S, D), BF16),
                pltpu.VMEM((D, 3 * D), BF16),
                pltpu.VMEM((D, D), BF16),
                pltpu.VMEM((D // 2, 3 * D), U32),
                pltpu.VMEM((D // 2, D), U32),
                pltpu.VMEM((D, F), BF16),
                pltpu.VMEM((F, D), BF16),
                pltpu.VMEM((8, F), F32),
                pltpu.VMEM((8, D), F32),
                pltpu.VMEM((S + R, D), F32),
                pltpu.VMEM((S + R + R // 2, D), F32),
                pltpu.VMEM((4 * D, 128), U32),
                pltpu.VMEM((3 * D // 2, R), U32),
                pltpu.VMEM((D, 128), U32),
                pltpu.VMEM((D, 128), U32),
                pltpu.VMEM((R // 2, D), U32),
                pltpu.VMEM((R // 2, F), U32),
                pltpu.VMEM((S, D), BF16),
                pltpu.VMEM((F,), BF16),
                pltpu.VMEM((D,), BF16),
                pltpu.SemaphoreType.DMA((NB,)),
                pltpu.SemaphoreType.DMA((3 * NG,)),
                pltpu.SemaphoreType.DMA((6,)),
                pltpu.SemaphoreType.DMA((NB, OC)),
                pltpu.SemaphoreType.DMA((2,)),
                pltpu.SemaphoreType.REGULAR,
            ],
            compiler_params=pltpu.CompilerParams(vmem_limit_bytes=110 * 1024 * 1024),
        )(A_x.reshape(S, D), A_wqkv, A_wo, B_w1, B_b1, B_w2, B_b2)
        return out.reshape(1, S, D)

    return run


@jax.jit
def pallas_interleave_layers__sliding_local_dilated__dense_activation_squared_relu__prompt_kernel(A_x, A_wqkv, A_wo, B_x, B_w1, B_b1, B_w2, B_b2):
    return make()(A_x, A_wqkv, A_wo, B_x, B_w1, B_b1, B_w2, B_b2)
```

```python
import functools

import numpy as np
import jax
import jax.numpy as jnp
from jax import lax
import jax.experimental.pallas as pl
import jax.experimental.pallas.tpu as pltpu

S, D, F, DH = 2048, 1024, 3584, 32
WIN, DIL = 8, 2
EPS = 1e-5
LAYERS = 2
F32, BF16, U32 = jnp.float32, jnp.bfloat16, jnp.uint32

R = 256
NB = S // R
GR = 128
GP = GR // 2
NG = D // GR
NH = DH // 8
LNC = 32
K1 = 5 * GR
OC = 4
WAITS = (0, 1, 2, 3, 4, 5, 6)
XN0 = S + R
QX0 = 3 * D
HI16 = np.uint32(0xFFFF0000)


def _dot(a, b):
    return jnp.dot(a, b, preferred_element_type=F32)


def _ln(x):
    m = jnp.mean(x, axis=-1, keepdims=True)
    c = x - m
    v = jnp.mean(c * c, axis=-1, keepdims=True)
    return c * lax.rsqrt(v + EPS)


def _pk(x):
    return pltpu.bitcast(x.astype(BF16), U32)


def _bf(w):
    return pltpu.bitcast(w, BF16)


def _unpack(w):
    return pltpu.bitcast(w << 16, F32), pltpu.bitcast(w & HI16, F32)


def _join(lo, hi):
    return (pltpu.bitcast(lo, U32) >> 16) | pltpu.bitcast(hi, U32)


def _round_join(lo, hi):
    r = jnp.concatenate([lo, hi], axis=0).astype(BF16).astype(F32)
    return _join(r[:8], r[8:])


def _rows(r, n):
    return pl.ds(r if isinstance(r, int) else pl.multiple_of(r, n), n)


def _blk(i):
    return _rows(i * R, R)


def _kernel(x_hbm, wqkv_hbm, wo_hbm, w1_hbm, b1_hbm, w2_hbm, b2_hbm, out_hbm,
            xin, wqkv, wo, wq32, wo32, w1, w2, bb1, bb2, xa, xb, qkv, qkv0, kprev, vprev, o, h,
            ostage, b1, b2, sem_x, sem_qkv, sem_w, sem_o, sem_c, sem_f):

    cp_q = [[pltpu.make_async_copy(wqkv_hbm.at[:, pl.ds(p * D + g * GR, GR)],
                                   wqkv.at[:, pl.ds(p * D + g * GR, GR)],
                                   sem_qkv.at[g * 3 + p]) for p in range(3)] for g in range(NG)]

    def cp_x(i):
        return pltpu.make_async_copy(x_hbm.at[_blk(i)], xin.at[_blk(i)], sem_x.at[i])

    def cp_o(i, c):
        cs = pl.ds(c * (D // OC), D // OC)
        return pltpu.make_async_copy(ostage.at[_blk(i), cs], out_hbm.at[_blk(i), cs], sem_o.at[i, c])

    cp_ba = pltpu.make_async_copy(xb.at[_blk(0)], xa.at[_blk(NB)], sem_c.at[0])
    cp_ab = pltpu.make_async_copy(xa.at[_blk(0)], xb.at[_blk(NB)], sem_c.at[1])
    cp_wo1 = pltpu.make_async_copy(wo_hbm.at[:K1], wo.at[:K1], sem_w.at[0])
    cp_wo2 = pltpu.make_async_copy(wo_hbm.at[K1:], wo.at[K1:], sem_w.at[3])
    cp_b1 = pltpu.make_async_copy(b1_hbm, b1, sem_w.at[4])
    cp_b2 = pltpu.make_async_copy(b2_hbm, b2, sem_w.at[5])
    cp_w1 = pltpu.make_async_copy(w1_hbm, w1, sem_w.at[1])
    cp_w2 = pltpu.make_async_copy(w2_hbm, w2, sem_w.at[2])

    cp_x(0).start()
    pl.semaphore_signal(sem_f)
    pl.semaphore_wait(sem_f)
    for c in cp_q[0] + [cp_b1, cp_b2]:
        c.start()

    def get_xn():
        return pltpu.bitcast(xb[pl.ds(XN0, R // 2), :], BF16)

    def load_x(src_ref, i, off, n, from_input):
        if from_input is True:
            return xin[_rows(i * R + off, n), :].astype(F32)
        sl = _rows(i * R + off, n)
        if from_input is False:
            return src_ref[sl, :]
        si = _rows(jnp.minimum(i, NB - 1) * R + off, n)
        return jnp.where(from_input, xin[si, :].astype(F32), src_ref[sl, :])

    def layernorm(src_ref, i, from_input=False, zero=0):
        for c in range(R // LNC):
            y = _ln(load_x(src_ref, i, c * LNC, LNC, from_input))
            xb[_rows(zero + XN0 + c * LNC // 2, LNC // 2), :] = pltpu.bitcast(y.astype(BF16), F32)

    def layernorm_staged(i, zero, from_input):
        for c in range(R // LNC):
            y = _pk(_ln(load_x(xa, i, c * LNC, LNC, from_input)))
            for k in range(D // 128):
                rows = _rows(zero + QX0 + k * (R // 2) + c * LNC // 2, LNC // 2)
                qkv[rows, :] = y[:, k * 128:(k + 1) * 128]

    def unstage():
        for k in range(D // 128):
            xb[pl.ds(XN0, R // 2), pl.ds(k * 128, 128)] = pltpu.bitcast(
                qkv[pl.ds(QX0 + k * (R // 2), R // 2), :], F32)

    lane = lax.broadcasted_iota(jnp.int32, (8, 128), 1)
    sub = lax.broadcasted_iota(jnp.int32, (8, 128), 0)
    m_even = (sub & 2) == 0
    m_odd = ((sub + 7) & 2) == 0
    m_par = (sub & 1) == 0

    def fold2(mask, a, b, shift):
        return jnp.where(mask, a, b) + pltpu.roll(jnp.where(mask, b, a), 8 - shift, 0)

    def softmax(lg):
        mx = jnp.maximum(jnp.maximum(jnp.maximum(lg[0], lg[1]), jnp.maximum(lg[2], lg[3])),
                         jnp.maximum(jnp.maximum(lg[4], lg[5]), jnp.maximum(lg[6], lg[7])))
        e = [jnp.exp(a - mx) for a in lg]
        inv = 1.0 / functools.reduce(jnp.add, e)
        return [a * inv for a in e]

    def attention(g, first):
        base = g * 3 * GR

        def shifted(part, prev_ref, d):
            cur = qkv[pl.ds(base + part * GR + d * 8, 8), :]
            out = [_unpack(cur)]
            prev = prev_ref[pl.ds(g * GR + d * 8, 8), :]
            if part == 2:
                b = jnp.broadcast_to(out[0][0][:, 0:1], (8, 128))
                prev = jnp.where(first, _join(b, b), prev)
            for w in range(1, WIN):
                out.append(_unpack(pltpu.roll(jnp.where(lane >= 128 - w, prev, cur), w, 1)))
            return out

        def probs(hp):
            half = []
            for hd in (2 * hp, 2 * hp + 1):
                acc = [[None, None] for _ in range(WIN)]
                for d in range(hd * NH, (hd + 1) * NH):
                    q = _unpack(qkv[pl.ds(base + d * 8, 8), :])
                    ks = shifted(1, kprev, d)
                    for k in range(2):
                        for w in range(WIN):
                            pr = q[k] * ks[w][k]
                            acc[w][k] = pr if acc[w][k] is None else acc[w][k] + pr
                half.append([fold2(m_odd if hd % 2 else m_even, a, b, 2) for a, b in acc])
            lg = []
            for u, v in zip(*half):
                z = fold2(m_par, u, v, 1)
                lg.append((z + pltpu.roll(z, 4, 0)) * (DH ** -0.5))
            lg = [lg[0]] + [jnp.where(jnp.logical_and(first, lane < w), -1e9, lg[w])
                            for w in range(1, WIN)]
            return softmax(lg)

        def values(hp, p):
            outs = []
            for hd in (2 * hp, 2 * hp + 1):
                ph = [[jnp.broadcast_to(a[hd % 2 + 2 * k:hd % 2 + 2 * k + 1, :], (8, 128))
                       for k in range(2)] for a in p]
                for d in range(hd * NH, (hd + 1) * NH):
                    vs = shifted(2, vprev, d)
                    res = []
                    for k in range(2):
                        acc = ph[WIN - 1][k] * vs[WIN - 1][k]
                        for w in range(WIN - 2, -1, -1):
                            acc = acc + ph[w][k] * vs[w][k]
                        res.append(acc)
                    outs.append(_round_join(*res))
            return outs

        ps = [probs(0), probs(1)]
        outs = values(0, ps[0]) + values(1, ps[1])
        o[:, pl.ds(g * GR, GR)] = jnp.concatenate(outs, axis=0).T
        kprev[pl.ds(g * GR, GR), :] = qkv[pl.ds(base + GR, GR), :]
        vprev[pl.ds(g * GR, GR), :] = qkv[pl.ds(base + 2 * GR, GR), :]

    def attention_first(g):
        base = g * 3 * GP
        for t in range(R // 128):
            cols = pl.ds(t * 128, 128)

            def shifted(part, d):
                rows = pl.ds(base + part * GP + d * 8, 8)
                cur = qkv0[rows, cols]
                if t == 0:
                    prev = jnp.broadcast_to(cur[:, 0:1], (8, 128))
                else:
                    prev = qkv0[rows, pl.ds((t - 1) * 128, 128)]
                out = [_unpack(cur)]
                for w in range(1, WIN):
                    sh = w * DIL
                    out.append(_unpack(pltpu.roll(jnp.where(lane >= 128 - sh, prev, cur), sh, 1)))
                return out

            acc = [[None] * 4 for _ in range(WIN)]
            for d in range(GP // 8):
                hd = d // 2
                q0, q1 = _unpack(qkv0[pl.ds(base + d * 8, 8), cols])
                ks = shifted(1, d)
                for w in range(WIN):
                    pr = q0 * ks[w][0] + q1 * ks[w][1]
                    acc[w][hd] = pr if acc[w][hd] is None else acc[w][hd] + pr
            lg = []
            for a in acc:
                z = fold2(m_par, fold2(m_even, a[0], a[2], 2), fold2(m_odd, a[1], a[3], 2), 1)
                lg.append((z + pltpu.roll(z, 4, 0)) * (DH ** -0.5))
            if t == 0:
                lg = [lg[0]] + [jnp.where(lane < w * DIL, -1e9, lg[w]) for w in range(1, WIN)]
            p = softmax(lg)
            outs = []
            for d in range(GP // 8):
                hd = d // 2
                if d % 2 == 0:
                    ph = [jnp.broadcast_to(a[hd:hd + 1, :], (8, 128)) for a in p]
                vs = shifted(2, d)
                res = []
                for k in range(2):
                    acc_o = ph[0] * vs[0][k]
                    for w in range(1, WIN):
                        acc_o = acc_o + ph[w] * vs[w][k]
                    res.append(acc_o)
                outs.append(_bf(_round_join(*res)))
            oT = jnp.concatenate(outs, axis=0)
            o[pl.ds(t * 64, 64), pl.ds(g * GR, GR)] = pltpu.bitcast(oT.T, U32)

    def first_unit():
        def finish_v(g):
            qkv0[pl.ds((g * 3 + 2) * GP, GP), :] = pltpu.bitcast(
                _bf(vprev[pl.ds(g * GR, GR), :]).T, U32)

        def need(g):
            if g not in WAITS:
                return
            for gg in range(g, min([w for w in WAITS if w > g] + [NG])):
                for c in cp_q[gg]:
                    c.wait()
            if g == 0:
                cp_wo1.start()
                cp_x(1).start()
                cp_wo2.start()
                cp_b1.wait()
                cp_b2.wait()
                bb1[...] = jnp.broadcast_to(b1[...].astype(F32).reshape(1, F), (8, F))
                bb2[...] = jnp.broadcast_to(b2[...].astype(F32).reshape(1, D), (8, D))
            else:
                finish_v(g - 1)

        def proj(g):
            for p in range(3):
                cs = pl.ds(p * D + g * GR, GR)
                wv = wqkv[:, cs]
                wq32[:, cs] = pltpu.bitcast(wv, U32)
                y = _pk(_dot(get_xn(), wv))
                if p:
                    (kprev, vprev)[p - 1][pl.ds(g * GR, GR), :] = y
                if not (p == 2 and (g + 1 in WAITS or g + 1 == NG)):
                    qkv0[pl.ds((g * 3 + p) * GP, GP), :] = pltpu.bitcast(_bf(y).T, U32)

        def get_wo(a, b):
            wv = wo[a:b, :]
            wo32[a // 2:b // 2, :] = pltpu.bitcast(wv, U32)
            return wv

        need(0)
        proj(0)
        for g in range(NG - 1):
            need(g + 1)
            attention_first(g)
            proj(g + 1)
        cp_wo1.wait()
        for j in range(2, NB):
            cp_x(j).start()
        finish_v(NG - 1)
        y = _dot(_bf(o[:, :K1]), get_wo(0, K1))
        xb[_blk(0), :] = load_x(xa, 0, 0, R, True) + y
        attention_first(NG - 1)
        cp_x(1).wait()
        cp_wo2.wait()
        cp_w1.start()
        cp_w2.start()
        layernorm(xa, 1, True, pl.program_id(0))
        for g in range(NG):
            for ref in (kprev, vprev):
                ref[pl.ds(g * GR, GR), :] = ref[pl.ds(g * GR, GR), :].T
        xb[_blk(0), :] = xb[_blk(0), :] + _dot(_bf(o[:, K1:]), get_wo(K1, D))

    def attn_unit(i, l):
        first = i == 0

        def proj(g):
            for p in range(3):
                if g == 0 and p == 1:
                    layernorm_staged(i + 1, i >> 8, jnp.logical_and(l == 0, i + 1 < NB))
                wv = _bf(wq32[:, pl.ds(p * D + g * GR, GR)])
                qkv[pl.ds((g * 3 + p) * GR, GR), :] = _pk(_dot(get_xn(), wv)).T

        proj(0)
        for g in range(NG - 1):
            proj(g + 1)
            attention(g, first)
        y = _dot(_bf(o[:, :K1]), _bf(wo32[:K1 // 2, :]))
        xb[_blk(i), :] = load_x(xa, i, 0, R, l == 0) + y
        attention(NG - 1, first)
        unstage()
        xb[_blk(i), :] = xb[_blk(i), :] + _dot(_bf(o[:, K1:]), _bf(wo32[K1 // 2:, :]))

    def ffn_unit(i, l):
        hh = _dot(get_xn(), w1[...]) + bb1[0:1, :]
        rr = jnp.where(hh > 0, hh, 0.0)
        h[...] = _pk(rr * rr)
        layernorm(xb, i + 1)
        for c in range(OC):
            cs = pl.ds(c * (D // OC), D // OC)
            x2 = xb[_blk(i), cs] + (_dot(_bf(h[...]), w2[:, cs]) + bb2[0:1, cs])
            xa[_blk(i), cs] = x2
            ostage[_blk(i), cs] = x2.astype(BF16)

            @pl.when(l == LAYERS - 1)
            def _():
                cp_o(i, c).start()

    cp_x(0).wait()
    for g in range(1, NG):
        for c in cp_q[g]:
            c.start()
    layernorm(xa, 0, True)
    first_unit()

    def layer(l, carry):
        def attn_step(i, c):
            @pl.when(jnp.logical_and(l == 0, i + 1 < NB))
            def _():
                cp_x(i + 1).wait()

            @pl.when(i == 1)
            def _():
                cp_ba.start()

            @pl.when(i == NB - 1)
            def _():
                cp_ba.wait()

            attn_unit(i, l)
            return c

        lax.fori_loop(jnp.where(l == 0, 1, 0), NB, attn_step, 0)

        @pl.when(l == 0)
        def _():
            cp_w1.wait()
            cp_w2.wait()

        def ffn_step(i, c):
            @pl.when(i == 1)
            def _():
                cp_ab.start()

            @pl.when(i == NB - 1)
            def _():
                cp_ab.wait()

            ffn_unit(i, l)
            return c

        lax.fori_loop(0, NB, ffn_step, 0)
        return carry

    lax.fori_loop(0, LAYERS, layer, 0)
    for i in range(NB):
        for c in range(OC):
            cp_o(i, c).wait()


@jax.jit
def pallas_interleave_layers__sliding_local_dilated__dense_activation_squared_relu__prompt_kernel(
    A_x: jax.Array,
    A_wqkv: jax.Array,
    A_wo: jax.Array,
    B_x: jax.Array,
    B_w1: jax.Array,
    B_b1: jax.Array,
    B_w2: jax.Array,
    B_b2: jax.Array,
):
    del B_x
    hbm = pl.BlockSpec(memory_space=pl.ANY)
    out = pl.pallas_call(
        _kernel,
        out_shape=jax.ShapeDtypeStruct((S, D), BF16),
        grid=(1,),
        in_specs=[hbm] * 7,
        out_specs=hbm,
        scratch_shapes=[
            pltpu.VMEM((S, D), BF16),
            pltpu.VMEM((D, 3 * D), BF16),
            pltpu.VMEM((D, D), BF16),
            pltpu.VMEM((D // 2, 3 * D), U32),
            pltpu.VMEM((D // 2, D), U32),
            pltpu.VMEM((D, F), BF16),
            pltpu.VMEM((F, D), BF16),
            pltpu.VMEM((8, F), F32),
            pltpu.VMEM((8, D), F32),
            pltpu.VMEM((S + R, D), F32),
            pltpu.VMEM((S + R + R // 2, D), F32),
            pltpu.VMEM((4 * D, 128), U32),
            pltpu.VMEM((3 * D // 2, R), U32),
            pltpu.VMEM((D, 128), U32),
            pltpu.VMEM((D, 128), U32),
            pltpu.VMEM((R // 2, D), U32),
            pltpu.VMEM((R // 2, F), U32),
            pltpu.VMEM((S, D), BF16),
            pltpu.VMEM((F,), BF16),
            pltpu.VMEM((D,), BF16),
            pltpu.SemaphoreType.DMA((NB,)),
            pltpu.SemaphoreType.DMA((3 * NG,)),
            pltpu.SemaphoreType.DMA((6,)),
            pltpu.SemaphoreType.DMA((NB, OC)),
            pltpu.SemaphoreType.DMA((2,)),
            pltpu.SemaphoreType.REGULAR,
        ],
        compiler_params=pltpu.CompilerParams(vmem_limit_bytes=110 * 1024 * 1024),
    )(A_x.reshape(S, D), A_wqkv, A_wo, B_w1, B_b1, B_w2, B_b2)
    return out.reshape(1, S, D)
```

```python
import contextlib
import functools

import numpy as np
import jax
import jax.numpy as jnp
from jax import lax
import jax.experimental.pallas as pl
import jax.experimental.pallas.tpu as pltpu

S, D, F, DH = 2048, 1024, 3584, 32
WIN, DIL = 8, 2
EPS = 1e-5
LAYERS = 2
F32, BF16, U32 = jnp.float32, jnp.bfloat16, jnp.uint32

R = 256
NB = S // R
GR = 128
GP = GR // 2
NG = D // GR
NH = DH // 8
LNC = 32
K1_ = 5 * GR
OC = D // 128
RH, DHF, FH = R // 2, D // 2, F // 2
WAITS = (0, 1, 2, 3, 4, 5, 6)
XN0 = S + R
XT0 = XN0 + R // 2
QX0 = 3 * D
SUMS = (0, 2, 3, 5, 6)
HI16 = np.uint32(0xFFFF0000)


def _dot(a, b):
    return jnp.dot(a, b, preferred_element_type=F32)


def _ln(x):
    m = jnp.mean(x, axis=-1, keepdims=True)
    c = x - m
    v = jnp.mean(c * c, axis=-1, keepdims=True)
    return c * lax.rsqrt(v + EPS)


def _pk(x):
    return pltpu.bitcast(x.astype(BF16), U32)


def _bf(w):
    return pltpu.bitcast(w, BF16)


def _unpack(w):
    return pltpu.bitcast(w << 16, F32), pltpu.bitcast(w & HI16, F32)


def _join(lo, hi):
    return (pltpu.bitcast(lo, U32) >> 16) | pltpu.bitcast(hi, U32)


def _round_join(lo, hi):
    r = jnp.concatenate([lo, hi], axis=0).astype(BF16).astype(F32)
    return _join(r[:8], r[8:])


def _lhs7(a11, a12, a21, a22):
    return [a11 + a22, a21 + a22, a11, a22, a11 + a12, a21 - a11, a12 - a22]


def _rhs5(*b):
    b11, b12, b21, b22 = (t.astype(F32) for t in b)
    return b11 + b22, b12 - b22, b21 - b11, b11 + b12, b21 + b22


def _seven(mul):
    m1, m4, m5, m7 = mul(0), mul(3), mul(4), mul(6)
    c11 = m1 + m4 - m5 + m7
    m2 = mul(1)
    c21 = m2 + m4
    m3 = mul(2)
    c12 = m3 + m5
    c22 = m1 - m2 + m3 + mul(5)
    return c11, c12, c21, c22


def _rows(r, n):
    return pl.ds(r if isinstance(r, int) else pl.multiple_of(r, n), n)


def _blk(i):
    return _rows(i * R, R)


def _kernel(x_hbm, wqkv_hbm, wo_hbm, w1_hbm, b1_hbm, w2_hbm, b2_hbm, out_hbm,
            xin, wqkv, wo, wq32, sq, wo32, w1, w2, s1, s2, bb1, bb2, xa, xb, qkv, qkv0, kprev, vprev, o, h,
            ostage, b1, b2, sem_x, sem_qkv, sem_w, sem_o, sem_c, sem_f, *, WOS, LNP, LNA, KO, PW, PR1, PR2, PS, NW1, NW2, LNF, SC, ONLY):

    K1 = WOS * GR
    cp_q = [[pltpu.make_async_copy(wqkv_hbm.at[:, pl.ds(p * D + g * GR, GR)],
                                   wqkv.at[:, pl.ds(p * D + g * GR, GR)],
                                   sem_qkv.at[g * 3 + p]) for p in range(3)] for g in range(NG)]

    def cp_x(i):
        return pltpu.make_async_copy(x_hbm.at[_blk(i)], xin.at[_blk(i)], sem_x.at[i])

    def cp_o(i, c):
        cs = pl.ds(c * (D // OC), D // OC)
        return pltpu.make_async_copy(ostage.at[_blk(i), cs], out_hbm.at[_blk(i), cs], sem_o.at[i, c])

    cp_ba = pltpu.make_async_copy(xb.at[_blk(0)], xa.at[_blk(NB)], sem_c.at[0])
    cp_ab = pltpu.make_async_copy(xa.at[_blk(0)], xb.at[_blk(NB)], sem_c.at[1])
    cp_wo1 = pltpu.make_async_copy(wo_hbm.at[:K1], wo.at[:K1], sem_w.at[0])
    cp_wo2 = pltpu.make_async_copy(wo_hbm.at[K1:], wo.at[K1:], sem_w.at[3])
    cp_b1 = pltpu.make_async_copy(b1_hbm, b1, sem_w.at[4])
    cp_b2 = pltpu.make_async_copy(b2_hbm, b2, sem_w.at[5])
    cp_w1 = pltpu.make_async_copy(w1_hbm, w1, sem_w.at[1])
    cp_w2 = pltpu.make_async_copy(w2_hbm, w2, sem_w.at[2])

    cp_x(0).start()
    pl.semaphore_signal(sem_f)
    pl.semaphore_wait(sem_f)
    for c in cp_q[0] + [cp_b1, cp_b2]:
        c.start()

    def get_xn():
        return pltpu.bitcast(xb[pl.ds(XN0, R // 2), :], BF16)

    def load_x(src_ref, i, off, n, from_input):
        if from_input is True:
            return xin[_rows(i * R + off, n), :].astype(F32)
        sl = _rows(i * R + off, n)
        if from_input is False:
            return src_ref[sl, :]
        si = _rows(jnp.minimum(i, NB - 1) * R + off, n)
        return jnp.where(from_input, xin[si, :].astype(F32), src_ref[sl, :])

    def layernorm(src_ref, i, from_input=False, zero=0):
        for c in range(R // LNC):
            y = _ln(load_x(src_ref, i, c * LNC, LNC, from_input))
            xb[_rows(zero + XN0 + c * LNC // 2, LNC // 2), :] = pltpu.bitcast(y.astype(BF16), F32)

    def xt(k, lo=0, n=RH // 2):
        return (XT0 + (k // 2) * (RH // 2) + lo, n), pl.ds((k % 2) * DHF, DHF)

    def get_xt(k):
        (r, n), c = xt(k)
        return pltpu.bitcast(xb[pl.ds(r, n), c], BF16)

    def ln7(src_ref, i, from_input, n):
        for c in range(RH // n):
            top = _ln(load_x(src_ref, i, c * n, n, from_input))
            bot = _ln(load_x(src_ref, i, RH + c * n, n, from_input))
            for k, t in enumerate(_lhs7(top[:, :DHF], top[:, DHF:], bot[:, :DHF], bot[:, DHF:])):
                yield c, k, t

    def layernorm7(src_ref, i, from_input=False, zero=0):
        for c, k, t in ln7(src_ref, i, from_input, LNF):
            (r, n), cs = xt(k, c * LNF // 2, LNF // 2)
            xb[_rows(zero + r, n), cs] = pltpu.bitcast(t.astype(BF16), F32)

    def layernorm_staged(i, zero, from_input):
        for c, k, t in ln7(xa, i, from_input, LNA):
            (r, n), cs = xt(k, c * LNA // 2, LNA // 2)
            o[_rows(zero + r - XT0 + RH, n), cs] = _pk(t)

    def unstage():
        for k in range(7):
            (r, n), cs = xt(k)
            xb[pl.ds(r, n), cs] = pltpu.bitcast(o[pl.ds(r - XT0 + RH, n), cs], F32)

    lane = lax.broadcasted_iota(jnp.int32, (8, 128), 1)
    sub = lax.broadcasted_iota(jnp.int32, (8, 128), 0)
    m_even = (sub & 2) == 0
    m_odd = ((sub + 7) & 2) == 0
    m_par = (sub & 1) == 0

    def fold2(mask, a, b, shift):
        return jnp.where(mask, a, b) + pltpu.roll(jnp.where(mask, b, a), 8 - shift, 0)

    def softmax(lg):
        mx = jnp.maximum(jnp.maximum(jnp.maximum(lg[0], lg[1]), jnp.maximum(lg[2], lg[3])),
                         jnp.maximum(jnp.maximum(lg[4], lg[5]), jnp.maximum(lg[6], lg[7])))
        e = [jnp.exp(a - mx) for a in lg]
        inv = 1.0 / functools.reduce(jnp.add, e)
        return [a * inv for a in e]

    def attention(g, first):
        base = g * 3 * GR

        def shifted(part, prev_ref, d):
            cur = qkv[pl.ds(base + part * GR + d * 8, 8), :]
            out = [_unpack(cur)]
            prev = prev_ref[pl.ds(g * GR + d * 8, 8), :]
            if part == 2:
                b = jnp.broadcast_to(out[0][0][:, 0:1], (8, 128))
                prev = jnp.where(first, _join(b, b), prev)
            for w in range(1, WIN):
                out.append(_unpack(pltpu.roll(jnp.where(lane >= 128 - w, prev, cur), w, 1)))
            return out

        def probs(hp):
            half = []
            for hd in (2 * hp, 2 * hp + 1):
                acc = [[None, None] for _ in range(WIN)]
                for d in range(hd * NH, (hd + 1) * NH):
                    q = _unpack(qkv[pl.ds(base + d * 8, 8), :])
                    ks = shifted(1, kprev, d)
                    for k in range(2):
                        for w in range(WIN):
                            pr = q[k] * ks[w][k]
                            acc[w][k] = pr if acc[w][k] is None else acc[w][k] + pr
                half.append([fold2(m_odd if hd % 2 else m_even, a, b, 2) for a, b in acc])
            lg = []
            for u, v in zip(*half):
                z = fold2(m_par, u, v, 1)
                lg.append((z + pltpu.roll(z, 4, 0)) * (DH ** -0.5))
            lg = [lg[0]] + [jnp.where(jnp.logical_and(first, lane < w), -1e9, lg[w])
                            for w in range(1, WIN)]
            return softmax(lg)

        def values(hp, p):
            outs = []
            for hd in (2 * hp, 2 * hp + 1):
                ph = [[jnp.broadcast_to(a[hd % 2 + 2 * k:hd % 2 + 2 * k + 1, :], (8, 128))
                       for k in range(2)] for a in p]
                for d in range(hd * NH, (hd + 1) * NH):
                    vs = shifted(2, vprev, d)
                    res = []
                    for k in range(2):
                        acc = ph[WIN - 1][k] * vs[WIN - 1][k]
                        for w in range(WIN - 2, -1, -1):
                            acc = acc + ph[w][k] * vs[w][k]
                        res.append(acc)
                    outs.append(_round_join(*res))
            return outs

        ps = [probs(0), probs(1)]
        outs = values(0, ps[0]) + values(1, ps[1])
        o[:RH, pl.ds(g * GR, GR)] = jnp.concatenate(outs, axis=0).T
        kprev[pl.ds(g * GR, GR), :] = qkv[pl.ds(base + GR, GR), :]
        vprev[pl.ds(g * GR, GR), :] = qkv[pl.ds(base + 2 * GR, GR), :]

    def attention_first(g):
        base = g * 3 * GP
        for t in range(R // 128):
            cols = pl.ds(t * 128, 128)

            def shifted(part, d):
                rows = pl.ds(base + part * GP + d * 8, 8)
                cur = qkv0[rows, cols]
                if t == 0:
                    prev = jnp.broadcast_to(cur[:, 0:1], (8, 128))
                else:
                    prev = qkv0[rows, pl.ds((t - 1) * 128, 128)]
                out = [_unpack(cur)]
                for w in range(1, WIN):
                    sh = w * DIL
                    out.append(_unpack(pltpu.roll(jnp.where(lane >= 128 - sh, prev, cur), sh, 1)))
                return out

            acc = [[None] * 4 for _ in range(WIN)]
            for d in range(GP // 8):
                hd = d // 2
                q0, q1 = _unpack(qkv0[pl.ds(base + d * 8, 8), cols])
                ks = shifted(1, d)
                for w in range(WIN):
                    pr = q0 * ks[w][0] + q1 * ks[w][1]
                    acc[w][hd] = pr if acc[w][hd] is None else acc[w][hd] + pr
            lg = []
            for a in acc:
                z = fold2(m_par, fold2(m_even, a[0], a[2], 2), fold2(m_odd, a[1], a[3], 2), 1)
                lg.append((z + pltpu.roll(z, 4, 0)) * (DH ** -0.5))
            if t == 0:
                lg = [lg[0]] + [jnp.where(lane < w * DIL, -1e9, lg[w]) for w in range(1, WIN)]
            p = softmax(lg)
            outs = []
            for d in range(GP // 8):
                hd = d // 2
                if d % 2 == 0:
                    ph = [jnp.broadcast_to(a[hd:hd + 1, :], (8, 128)) for a in p]
                vs = shifted(2, d)
                res = []
                for k in range(2):
                    acc_o = ph[0] * vs[0][k]
                    for w in range(1, WIN):
                        acc_o = acc_o + ph[w] * vs[w][k]
                    res.append(acc_o)
                outs.append(_bf(_round_join(*res)))
            oT = jnp.concatenate(outs, axis=0)
            o[pl.ds(t * 64, 64), pl.ds(g * GR, GR)] = pltpu.bitcast(oT.T, U32)

    def first_unit():
        def finish_v(g):
            qkv0[pl.ds((g * 3 + 2) * GP, GP), :] = pltpu.bitcast(
                _bf(vprev[pl.ds(g * GR, GR), :]).T, U32)

        def need(g):
            if g not in WAITS:
                return
            for gg in range(g, min([w for w in WAITS if w > g] + [NG])):
                for c in cp_q[gg]:
                    c.wait()
            if g == 0:
                cp_wo1.start()
                cp_x(1).start()
                cp_wo2.start()
                cp_b1.wait()
                cp_b2.wait()
                bb1[...] = jnp.broadcast_to(b1[...].astype(F32).reshape(1, F), (8, F))
                bb2[...] = jnp.broadcast_to(b2[...].astype(F32).reshape(1, D), (8, D))
            else:
                finish_v(g - 1)

        def proj(g):
            for p in range(3):
                cs = pl.ds(p * D + g * GR, GR)
                wv = wqkv[:, cs]
                wq32[:, cs] = pltpu.bitcast(wv, U32)
                y = _pk(_dot(get_xn(), wv))
                if p:
                    (kprev, vprev)[p - 1][pl.ds(g * GR, GR), :] = y
                if not (p == 2 and (g + 1 in WAITS or g + 1 == NG)):
                    qkv0[pl.ds((g * 3 + p) * GP, GP), :] = pltpu.bitcast(_bf(y).T, U32)

        def prepare_q(G, half=None):
            for p in range(3):
                c0, c1 = pl.ds(p * D + 2 * G * GR, GR), pl.ds(p * D + (2 * G + 1) * GR, GR)
                dst = pl.ds((G * 3 + p) * GR, GR)
                for r in range(0, DHF, PS) if half is None else range(half * DHF // 2, (half + 1) * DHF // 2, PS):
                    top, bot = pl.ds(r // 2, PS // 2), pl.ds((DHF + r) // 2, PS // 2)
                    for k, t in enumerate(_rhs5(_bf(wq32[top, c0]), _bf(wq32[top, c1]),
                                                _bf(wq32[bot, c0]), _bf(wq32[bot, c1]))):
                        sq[_rows(k * (DHF // 2) + (c * 16 if PW == 6 else r // 2), 16 if PW == 6 else PS // 2), dst] = _pk(t)

        def get_wo(a, b):
            wv = wo[a:b, :]
            wo32[a // 2:b // 2, :] = pltpu.bitcast(wv, U32)
            return wv

        need(0)
        proj(0)
        for g in range(NG - 1):
            need(g + 1)
            attention_first(g)
            proj(g + 1)
            if PW == 5 and g >= 2:
                prepare_q((g - 2) // 2, (g - 2) % 2)
        cp_wo1.wait()
        for j in range(2, NB):
            cp_x(j).start()
        finish_v(NG - 1)
        y = _dot(_bf(o[:RH, :K1]), get_wo(0, K1))
        if PW == 5:
            prepare_q(2, 1)
        for G in {5: (3,), 6: (), 0: (3,), 1: (0, 1, 2, 3), 2: (0, 1), 3: (), 4: (0, 1, 2, 3)}[PW]:
            prepare_q(G)
        xb[_blk(0), :] = load_x(xa, 0, 0, R, True) + y
        attention_first(NG - 1)
        cp_x(1).wait()
        cp_wo2.wait()
        cp_w1.start()
        cp_w2.start()
        layernorm7(xa, 1, True, pl.program_id(0))
        for G in {2: (2, 3), 3: (0, 1, 2, 3)}.get(PW, ()):
            prepare_q(G)
        for g in range(NG):
            for ref in (kprev, vprev):
                ref[pl.ds(g * GR, GR), :] = ref[pl.ds(g * GR, GR), :].T
        xb[_blk(0), :] = xb[_blk(0), :] + _dot(_bf(o[:RH, K1:]), get_wo(K1, D))

    def attn_unit(i, l):
        first = i == 0

        def proj(G):
            for n, p in enumerate(KO):
                if G * 3 + n == LNP:
                    layernorm_staged(i + 1, i >> 8, jnp.logical_and(l == 0, i + 1 < NB))
                cs = pl.ds((G * 3 + p) * GR, GR)

                def rhs_q(k):
                    if k == 1:
                        return wq32[:DHF // 2, pl.ds(p * D + 2 * G * GR, GR)]
                    if k == 4:
                        return wq32[DHF // 2:, pl.ds(p * D + (2 * G + 1) * GR, GR)]
                    return sq[pl.ds(SUMS.index(k) * (DHF // 2), DHF // 2), cs]

                c11, c12, c21, c22 = _seven(lambda k: _dot(get_xt(k), _bf(rhs_q(k))))
                for g, t, b in ((2 * G, c11, c21), (2 * G + 1, c12, c22)):
                    qkv[pl.ds((g * 3 + p) * GR, GR), :] = _pk(jnp.concatenate([t, b], axis=0)).T

        proj(0)
        for G in range(NG // 2 - 1):
            proj(G + 1)
            attention(2 * G, first)
            attention(2 * G + 1, first)
        y = _dot(_bf(o[:RH, :K1]), _bf(wo32[:K1 // 2, :]))
        xb[_blk(i), :] = load_x(xa, i, 0, R, l == 0) + y
        attention(NG - 2, first)
        attention(NG - 1, first)
        unstage()
        xb[_blk(i), :] = xb[_blk(i), :] + _dot(_bf(o[:RH, K1:]), _bf(wo32[K1 // 2:, :]))

    def prepare(w, sums, kh, nh, step):
        def body(c, carry):
            top, bot = _rows(c * step, step), _rows(kh + c * step, step)
            for j in range(0, nh, 256):
                c0, c1 = pl.ds(j, 256), pl.ds(nh + j, 256)
                for k, t in enumerate(_rhs5(w[top, c0], w[top, c1], w[bot, c0], w[bot, c1])):
                    sums[k, top, c0] = t.astype(BF16)
            return carry
        lax.fori_loop(0, kh // step, body, 0)

    def rhs(w, sums, k, kh, nh, j, n):
        if k == 1:
            return w[:kh, pl.ds(j, n)]
        if k == 4:
            return w[kh:, pl.ds(nh + j, n)]
        return sums[SUMS.index(k), :, pl.ds(j, n)]

    def ffn_unit(i, l):
        for j in range(0, FH, NW1):
            cs, cs2 = pl.ds(j, NW1), pl.ds(FH + j, NW1)

            def mul1(k):
                return _dot(get_xt(k), rhs(w1, s1, k, DHF, FH, j, NW1))

            hs = []
            for c, bias in zip(_seven(mul1), (cs, cs2, cs, cs2)):
                hh = c + bb1[0:1, bias]
                rr = jnp.where(hh > 0, hh, 0.0)
                hs.append(rr * rr)
            for k, t in enumerate(_lhs7(*hs)):
                h[pl.ds(k * (RH // 2), RH // 2), cs] = _pk(t)
        layernorm7(xb, i + 1)
        for j in range(0, DHF, NW2):
            cs = pl.ds(j, NW2)
            ys = _seven(lambda k: _dot(_bf(h[pl.ds(k * (RH // 2), RH // 2), :]), rhs(w2, s2, k, FH, DHF, j, NW2)))
            for y, r, c in zip(ys, (0, 0, RH, RH), (j, DHF + j, j, DHF + j)):
                rows, cc = _rows(i * R + r, RH), pl.ds(c, NW2)
                x2 = xb[rows, cc] + (y + bb2[0:1, cc])
                xa[rows, cc] = x2
                ostage[rows, cc] = x2.astype(BF16)

            @pl.when(l == LAYERS - 1)
            def _():
                for c in range(j // 128, (j + NW2) // 128):
                    cp_o(i, c).start()
                    cp_o(i, DHF // 128 + c).start()

    cp_x(0).wait()
    for g in range(1, NG):
        for c in cp_q[g]:
            c.start()
    layernorm(xa, 0, True)
    if ONLY in (None, 'P'):
        first_unit()
    if PW == 6:
        def body(c, carry):
            top, bot = _rows(c * 16, 16), _rows(DHF // 2 + c * 16, 16)
            for G in range(NG // 2):
                for p in range(3):
                    c0, c1 = pl.ds(p * D + 2 * G * GR, GR), pl.ds(p * D + (2 * G + 1) * GR, GR)
                    dst = pl.ds((G * 3 + p) * GR, GR)
                    for k, t in enumerate(_rhs5(_bf(wq32[top, c0]), _bf(wq32[top, c1]),
                                                _bf(wq32[bot, c0]), _bf(wq32[bot, c1]))):
                        sq[_rows(k * (DHF // 2) + (c * 16 if PW == 6 else r // 2), 16 if PW == 6 else PS // 2), dst] = _pk(t)
            return carry
        lax.fori_loop(0, DHF // 32, body, 0)

    def layer(l, carry):
        def attn_step(i, c):
            @pl.when(jnp.logical_and(l == 0, i + 1 < NB))
            def _():
                cp_x(i + 1).wait()

            @pl.when(i == 1)
            def _():
                cp_ba.start()

            @pl.when(i == NB - 1)
            def _():
                cp_ba.wait()

            with jax.named_scope("attn_unit") if SC else contextlib.nullcontext():
                attn_unit(i, l)
            return c

        if ONLY in (None, 'A'):
            lax.fori_loop(jnp.where(l == 0, 1, 0), NB, attn_step, 0)

        @pl.when(l == 0)
        def _():
            cp_w1.wait()
            cp_w2.wait()
            prepare(w1, s1, DHF, FH, PR1)
            prepare(w2, s2, FH, DHF, PR2)

        def ffn_step(i, c):
            @pl.when(i == 1)
            def _():
                cp_ab.start()

            @pl.when(i == NB - 1)
            def _():
                cp_ab.wait()

            with jax.named_scope("ffn_unit") if SC else contextlib.nullcontext():
                ffn_unit(i, l)
            return c

        if ONLY in (None, 'B'):
            lax.fori_loop(0, NB, ffn_step, 0)
        return carry

    lax.fori_loop(0, LAYERS, layer, 0)
    for i in range(NB):
        for c in range(OC):
            cp_o(i, c).wait()


def make(NW1=128, NW2=256, LNF=16, WOS=5, LNP=1, LNA=16, KO=(0, 1, 2), PW=5, PS=64, PR1=16, PR2=32, SC=False, ONLY=None):
  def run(A_x, A_wqkv, A_wo, B_x, B_w1, B_b1, B_w2, B_b2):
    del B_x
    hbm = pl.BlockSpec(memory_space=pl.ANY)
    out = pl.pallas_call(
        functools.partial(_kernel, WOS=WOS, LNP=LNP, LNA=LNA, KO=KO, PW=PW, PR1=PR1, PR2=PR2, PS=PS, NW1=NW1, NW2=NW2, LNF=LNF, SC=SC, ONLY=ONLY),
        out_shape=jax.ShapeDtypeStruct((S, D), BF16),
        grid=(1,),
        in_specs=[hbm] * 7,
        out_specs=hbm,
        scratch_shapes=[
            pltpu.VMEM((S, D), BF16),
            pltpu.VMEM((D, 3 * D), BF16),
            pltpu.VMEM((D, D), BF16),
            pltpu.VMEM((D // 2, 3 * D), U32),
            pltpu.VMEM((5 * DHF // 2, 3 * DHF), U32),
            pltpu.VMEM((D // 2, D), U32),
            pltpu.VMEM((D, F), BF16),
            pltpu.VMEM((F, D), BF16),
            pltpu.VMEM((5, DHF, FH), BF16),
            pltpu.VMEM((5, FH, DHF), BF16),
            pltpu.VMEM((8, F), F32),
            pltpu.VMEM((8, D), F32),
            pltpu.VMEM((S + R, D), F32),
            pltpu.VMEM((S + 2 * R + R // 2, D), F32),
            pltpu.VMEM((3 * D, 128), U32),
            pltpu.VMEM((3 * D // 2, R), U32),
            pltpu.VMEM((D, 128), U32),
            pltpu.VMEM((D, 128), U32),
            pltpu.VMEM((3 * RH, D), U32),
            pltpu.VMEM((7 * RH // 2, FH), U32),
            pltpu.VMEM((S, D), BF16),
            pltpu.VMEM((F,), BF16),
            pltpu.VMEM((D,), BF16),
            pltpu.SemaphoreType.DMA((NB,)),
            pltpu.SemaphoreType.DMA((3 * NG,)),
            pltpu.SemaphoreType.DMA((6,)),
            pltpu.SemaphoreType.DMA((NB, OC)),
            pltpu.SemaphoreType.DMA((2,)),
            pltpu.SemaphoreType.REGULAR,
        ],
        compiler_params=pltpu.CompilerParams(vmem_limit_bytes=120 * 1024 * 1024),
    )(A_x.reshape(S, D), A_wqkv, A_wo, B_w1, B_b1, B_w2, B_b2)
    return out.reshape(1, S, D)
  return run


@jax.jit
def pallas_interleave_layers__sliding_local_dilated__dense_activation_squared_relu__prompt_kernel(A_x, A_wqkv, A_wo, B_x, B_w1, B_b1, B_w2, B_b2):
    return make(LNP=2)(A_x, A_wqkv, A_wo, B_x, B_w1, B_b1, B_w2, B_b2)
```

```python
import functools

import numpy as np
import jax
import jax.numpy as jnp
from jax import lax
import jax.experimental.pallas as pl
import jax.experimental.pallas.tpu as pltpu

S, D, F, DH = 2048, 1024, 3584, 32
WIN, DIL = 8, 2
EPS = 1e-5
LAYERS = 2
F32, BF16, U32 = jnp.float32, jnp.bfloat16, jnp.uint32

R = 256
NB = S // R
GR = 128
GP = GR // 2
NG = D // GR
NH = DH // 8
LNC = 32
LN7 = 16
K1 = 5 * GR
OC = D // 128
RH, DHF, FH = R // 2, D // 2, F // 2
WH = RH // 2
WAITS = (0, 1, 2, 3, 4, 5, 6)
XN0 = S + R
XT0 = XN0 + RH
SUMS = (0, 2, 3, 5, 6)
HI16 = np.uint32(0xFFFF0000)


def _dot(a, b):
    return jnp.dot(a, b, preferred_element_type=F32)


def _ln(x):
    m = jnp.mean(x, axis=-1, keepdims=True)
    c = x - m
    v = jnp.mean(c * c, axis=-1, keepdims=True)
    return c * lax.rsqrt(v + EPS)


def _pk(x):
    return pltpu.bitcast(x.astype(BF16), U32)


def _bf(w):
    return pltpu.bitcast(w, BF16)


def _unpack(w):
    return pltpu.bitcast(w << 16, F32), pltpu.bitcast(w & HI16, F32)


def _join(lo, hi):
    return (pltpu.bitcast(lo, U32) >> 16) | pltpu.bitcast(hi, U32)


def _round_join(lo, hi):
    r = jnp.concatenate([lo, hi], axis=0).astype(BF16).astype(F32)
    return _join(r[:8], r[8:])


def _lhs7(a11, a12, a21, a22):
    return [a11 + a22, a21 + a22, a11, a22, a11 + a12, a21 - a11, a12 - a22]


def _rhs5(*b):
    b11, b12, b21, b22 = (t.astype(F32) for t in b)
    return b11 + b22, b12 - b22, b21 - b11, b11 + b12, b21 + b22


def _seven(mul):
    m1, m4, m5, m7 = mul(0), mul(3), mul(4), mul(6)
    c11 = m1 + m4 - m5 + m7
    m2 = mul(1)
    c21 = m2 + m4
    m3 = mul(2)
    c12 = m3 + m5
    c22 = m1 - m2 + m3 + mul(5)
    return c11, c12, c21, c22


def _rows(r, n):
    return pl.ds(r if isinstance(r, int) else pl.multiple_of(r, n), n)


def _blk(i):
    return _rows(i * R, R)


def _kernel(x_hbm, wqkv_hbm, wo_hbm, w1_hbm, b1_hbm, w2_hbm, b2_hbm, out_hbm,
            xin, wqkv, wo, wq32, sq, wo32, w1, w2, s1, s2, bb1, bb2, xa, xb, qkv, qkv0, kprev, vprev, o, h,
            ostage, b1, b2, sem_x, sem_qkv, sem_w, sem_o, sem_c, sem_f):

    cp_q = [[pltpu.make_async_copy(wqkv_hbm.at[:, pl.ds(p * D + g * GR, GR)],
                                   wqkv.at[:, pl.ds(p * D + g * GR, GR)],
                                   sem_qkv.at[g * 3 + p]) for p in range(3)] for g in range(NG)]

    def cp_x(i):
        return pltpu.make_async_copy(x_hbm.at[_blk(i)], xin.at[_blk(i)], sem_x.at[i])

    def cp_o(i, c):
        cs = pl.ds(c * (D // OC), D // OC)
        return pltpu.make_async_copy(ostage.at[_blk(i), cs], out_hbm.at[_blk(i), cs], sem_o.at[i, c])

    cp_ba = pltpu.make_async_copy(xb.at[_blk(0)], xa.at[_blk(NB)], sem_c.at[0])
    cp_ab = pltpu.make_async_copy(xa.at[_blk(0)], xb.at[_blk(NB)], sem_c.at[1])
    cp_wo1 = pltpu.make_async_copy(wo_hbm.at[:K1], wo.at[:K1], sem_w.at[0])
    cp_wo2 = pltpu.make_async_copy(wo_hbm.at[K1:], wo.at[K1:], sem_w.at[3])
    cp_b1 = pltpu.make_async_copy(b1_hbm, b1, sem_w.at[4])
    cp_b2 = pltpu.make_async_copy(b2_hbm, b2, sem_w.at[5])
    cp_w1 = pltpu.make_async_copy(w1_hbm, w1, sem_w.at[1])
    cp_w2 = pltpu.make_async_copy(w2_hbm, w2, sem_w.at[2])

    cp_x(0).start()
    pl.semaphore_signal(sem_f)
    pl.semaphore_wait(sem_f)
    for c in cp_q[0] + [cp_b1, cp_b2]:
        c.start()

    def get_xn():
        return pltpu.bitcast(xb[pl.ds(XN0, R // 2), :], BF16)

    def load_x(src_ref, i, off, n, from_input):
        if from_input is True:
            return xin[_rows(i * R + off, n), :].astype(F32)
        sl = _rows(i * R + off, n)
        if from_input is False:
            return src_ref[sl, :]
        si = _rows(jnp.minimum(i, NB - 1) * R + off, n)
        return jnp.where(from_input, xin[si, :].astype(F32), src_ref[sl, :])

    def layernorm_first():
        for c in range(R // LNC):
            y = _ln(load_x(xa, 0, c * LNC, LNC, True))
            xb[pl.ds(XN0 + c * LNC // 2, LNC // 2), :] = pltpu.bitcast(y.astype(BF16), F32)

    def xt(k):
        return (k // 2) * WH, pl.ds((k % 2) * DHF, DHF)

    def get_xt(k):
        r, cs = xt(k)
        return pltpu.bitcast(xb[pl.ds(XT0 + r, WH), cs], BF16)

    def ln7(src_ref, i, from_input):
        for c in range(RH // LN7):
            top = _ln(load_x(src_ref, i, c * LN7, LN7, from_input))
            bot = _ln(load_x(src_ref, i, RH + c * LN7, LN7, from_input))
            for k, t in enumerate(_lhs7(top[:, :DHF], top[:, DHF:], bot[:, :DHF], bot[:, DHF:])):
                r, cs = xt(k)
                yield r + c * LN7 // 2, cs, t

    def layernorm(src_ref, i, from_input=False, zero=0):
        for r, cs, t in ln7(src_ref, i, from_input):
            xb[_rows(zero + XT0 + r, LN7 // 2), cs] = pltpu.bitcast(t.astype(BF16), F32)

    def layernorm_staged(i, zero, from_input):
        for r, cs, t in ln7(xa, i, from_input):
            o[_rows(zero + RH + r, LN7 // 2), cs] = _pk(t)

    def unstage():
        for k in range(7):
            r, cs = xt(k)
            xb[pl.ds(XT0 + r, WH), cs] = pltpu.bitcast(o[pl.ds(RH + r, WH), cs], F32)

    lane = lax.broadcasted_iota(jnp.int32, (8, 128), 1)
    sub = lax.broadcasted_iota(jnp.int32, (8, 128), 0)
    m_even = (sub & 2) == 0
    m_odd = ((sub + 7) & 2) == 0
    m_par = (sub & 1) == 0

    def fold2(mask, a, b, shift):
        return jnp.where(mask, a, b) + pltpu.roll(jnp.where(mask, b, a), 8 - shift, 0)

    def softmax(lg):
        mx = jnp.maximum(jnp.maximum(jnp.maximum(lg[0], lg[1]), jnp.maximum(lg[2], lg[3])),
                         jnp.maximum(jnp.maximum(lg[4], lg[5]), jnp.maximum(lg[6], lg[7])))
        e = [jnp.exp(a - mx) for a in lg]
        inv = 1.0 / functools.reduce(jnp.add, e)
        return [a * inv for a in e]

    def attention(g, first):
        base = g * 3 * GR

        def shifted(part, prev_ref, d):
            cur = qkv[pl.ds(base + part * GR + d * 8, 8), :]
            out = [_unpack(cur)]
            prev = prev_ref[pl.ds(g * GR + d * 8, 8), :]
            if part == 2:
                b = jnp.broadcast_to(out[0][0][:, 0:1], (8, 128))
                prev = jnp.where(first, _join(b, b), prev)
            for w in range(1, WIN):
                out.append(_unpack(pltpu.roll(jnp.where(lane >= 128 - w, prev, cur), w, 1)))
            return out

        def probs(hp):
            half = []
            for hd in (2 * hp, 2 * hp + 1):
                acc = [[None, None] for _ in range(WIN)]
                for d in range(hd * NH, (hd + 1) * NH):
                    q = _unpack(qkv[pl.ds(base + d * 8, 8), :])
                    ks = shifted(1, kprev, d)
                    for k in range(2):
                        for w in range(WIN):
                            pr = q[k] * ks[w][k]
                            acc[w][k] = pr if acc[w][k] is None else acc[w][k] + pr
                half.append([fold2(m_odd if hd % 2 else m_even, a, b, 2) for a, b in acc])
            lg = []
            for u, v in zip(*half):
                z = fold2(m_par, u, v, 1)
                lg.append((z + pltpu.roll(z, 4, 0)) * (DH ** -0.5))
            lg = [lg[0]] + [jnp.where(jnp.logical_and(first, lane < w), -1e9, lg[w])
                            for w in range(1, WIN)]
            return softmax(lg)

        def values(hp, p):
            outs = []
            for hd in (2 * hp, 2 * hp + 1):
                ph = [[jnp.broadcast_to(a[hd % 2 + 2 * k:hd % 2 + 2 * k + 1, :], (8, 128))
                       for k in range(2)] for a in p]
                for d in range(hd * NH, (hd + 1) * NH):
                    vs = shifted(2, vprev, d)
                    res = []
                    for k in range(2):
                        acc = ph[WIN - 1][k] * vs[WIN - 1][k]
                        for w in range(WIN - 2, -1, -1):
                            acc = acc + ph[w][k] * vs[w][k]
                        res.append(acc)
                    outs.append(_round_join(*res))
            return outs

        ps = [probs(0), probs(1)]
        outs = values(0, ps[0]) + values(1, ps[1])
        o[:RH, pl.ds(g * GR, GR)] = jnp.concatenate(outs, axis=0).T
        kprev[pl.ds(g * GR, GR), :] = qkv[pl.ds(base + GR, GR), :]
        vprev[pl.ds(g * GR, GR), :] = qkv[pl.ds(base + 2 * GR, GR), :]

    def attention_first(g):
        base = g * 3 * GP
        for t in range(R // 128):
            cols = pl.ds(t * 128, 128)

            def shifted(part, d):
                rows = pl.ds(base + part * GP + d * 8, 8)
                cur = qkv0[rows, cols]
                if t == 0:
                    prev = jnp.broadcast_to(cur[:, 0:1], (8, 128))
                else:
                    prev = qkv0[rows, pl.ds((t - 1) * 128, 128)]
                out = [_unpack(cur)]
                for w in range(1, WIN):
                    sh = w * DIL
                    out.append(_unpack(pltpu.roll(jnp.where(lane >= 128 - sh, prev, cur), sh, 1)))
                return out

            acc = [[None] * 4 for _ in range(WIN)]
            for d in range(GP // 8):
                hd = d // 2
                q0, q1 = _unpack(qkv0[pl.ds(base + d * 8, 8), cols])
                ks = shifted(1, d)
                for w in range(WIN):
                    pr = q0 * ks[w][0] + q1 * ks[w][1]
                    acc[w][hd] = pr if acc[w][hd] is None else acc[w][hd] + pr
            lg = []
            for a in acc:
                z = fold2(m_par, fold2(m_even, a[0], a[2], 2), fold2(m_odd, a[1], a[3], 2), 1)
                lg.append((z + pltpu.roll(z, 4, 0)) * (DH ** -0.5))
            if t == 0:
                lg = [lg[0]] + [jnp.where(lane < w * DIL, -1e9, lg[w]) for w in range(1, WIN)]
            p = softmax(lg)
            outs = []
            for d in range(GP // 8):
                hd = d // 2
                if d % 2 == 0:
                    ph = [jnp.broadcast_to(a[hd:hd + 1, :], (8, 128)) for a in p]
                vs = shifted(2, d)
                res = []
                for k in range(2):
                    acc_o = ph[0] * vs[0][k]
                    for w in range(1, WIN):
                        acc_o = acc_o + ph[w] * vs[w][k]
                    res.append(acc_o)
                outs.append(_bf(_round_join(*res)))
            oT = jnp.concatenate(outs, axis=0)
            o[pl.ds(t * 64, 64), pl.ds(g * GR, GR)] = pltpu.bitcast(oT.T, U32)

    def first_unit():
        def finish_v(g):
            qkv0[pl.ds((g * 3 + 2) * GP, GP), :] = pltpu.bitcast(
                _bf(vprev[pl.ds(g * GR, GR), :]).T, U32)

        def need(g):
            if g not in WAITS:
                return
            for gg in range(g, min([w for w in WAITS if w > g] + [NG])):
                for c in cp_q[gg]:
                    c.wait()
            if g == 0:
                cp_wo1.start()
                cp_x(1).start()
                cp_wo2.start()
                cp_b1.wait()
                cp_b2.wait()
                bb1[...] = jnp.broadcast_to(b1[...].astype(F32).reshape(1, F), (8, F))
                bb2[...] = jnp.broadcast_to(b2[...].astype(F32).reshape(1, D), (8, D))
            else:
                finish_v(g - 1)

        def proj(g):
            for p in range(3):
                cs = pl.ds(p * D + g * GR, GR)
                wv = wqkv[:, cs]
                wq32[:, cs] = pltpu.bitcast(wv, U32)
                y = _pk(_dot(get_xn(), wv))
                if p:
                    (kprev, vprev)[p - 1][pl.ds(g * GR, GR), :] = y
                if not (p == 2 and (g + 1 in WAITS or g + 1 == NG)):
                    qkv0[pl.ds((g * 3 + p) * GP, GP), :] = pltpu.bitcast(_bf(y).T, U32)

        def prepare_q(G, half):
            for p in range(3):
                c0, c1 = pl.ds(p * D + 2 * G * GR, GR), pl.ds(p * D + (2 * G + 1) * GR, GR)
                for r in range(half * DHF // 4, (half + 1) * DHF // 4, 32):
                    top, bot = pl.ds(r, 32), pl.ds(DHF // 2 + r, 32)
                    for k, t in enumerate(_rhs5(_bf(wq32[top, c0]), _bf(wq32[top, c1]),
                                                _bf(wq32[bot, c0]), _bf(wq32[bot, c1]))):
                        sq[pl.ds(k * (DHF // 2) + r, 32), pl.ds((G * 3 + p) * GR, GR)] = _pk(t)

        def get_wo(a, b):
            wv = wo[a:b, :]
            wo32[a // 2:b // 2, :] = pltpu.bitcast(wv, U32)
            return wv

        need(0)
        proj(0)
        for g in range(NG - 1):
            need(g + 1)
            attention_first(g)
            proj(g + 1)
            if g >= 1:
                prepare_q((g - 1) // 2, (g - 1) % 2)
        cp_wo1.wait()
        cp_x(1).wait()
        cp_wo2.wait()
        for j in range(2, NB):
            cp_x(j).start()
        finish_v(NG - 1)
        y = _dot(_bf(o[:RH, :K1]), get_wo(0, K1))
        prepare_q(3, 0)
        prepare_q(3, 1)
        xb[_blk(0), :] = load_x(xa, 0, 0, R, True) + y
        attention_first(NG - 1)
        cp_w1.start()
        cp_w2.start()
        layernorm(xa, 1, True, pl.program_id(0))
        for g in range(NG):
            for ref in (kprev, vprev):
                ref[pl.ds(g * GR, GR), :] = ref[pl.ds(g * GR, GR), :].T
        xb[_blk(0), :] = xb[_blk(0), :] + _dot(_bf(o[:RH, K1:]), get_wo(K1, D))

    def attn_unit(i, l):
        first = i == 0

        def proj(G):
            for p in range(3):
                if G == 0 and p == 2:
                    layernorm_staged(i + 1, i >> 8, jnp.logical_and(l == 0, i + 1 < NB))

                def rhs_q(k):
                    if k == 1:
                        return wq32[:DHF // 2, pl.ds(p * D + 2 * G * GR, GR)]
                    if k == 4:
                        return wq32[DHF // 2:, pl.ds(p * D + (2 * G + 1) * GR, GR)]
                    return sq[pl.ds(SUMS.index(k) * (DHF // 2), DHF // 2), pl.ds((G * 3 + p) * GR, GR)]

                c11, c12, c21, c22 = _seven(lambda k: _dot(get_xt(k), _bf(rhs_q(k))))
                for g, t, b in ((2 * G, c11, c21), (2 * G + 1, c12, c22)):
                    qkv[pl.ds((g * 3 + p) * GR, GR), :] = _pk(jnp.concatenate([t, b], axis=0)).T

        proj(0)
        for G in range(NG // 2 - 1):
            proj(G + 1)
            attention(2 * G, first)
            attention(2 * G + 1, first)
        y = _dot(_bf(o[:RH, :K1]), _bf(wo32[:K1 // 2, :]))
        xb[_blk(i), :] = load_x(xa, i, 0, R, l == 0) + y
        attention(NG - 2, first)
        attention(NG - 1, first)
        unstage()
        xb[_blk(i), :] = xb[_blk(i), :] + _dot(_bf(o[:RH, K1:]), _bf(wo32[K1 // 2:, :]))

    def prepare(w, sums, kh, nh, step):
        def body(c, carry):
            top, bot = _rows(c * step, step), _rows(kh + c * step, step)
            for j in range(0, nh, 256):
                c0, c1 = pl.ds(j, 256), pl.ds(nh + j, 256)
                for k, t in enumerate(_rhs5(w[top, c0], w[top, c1], w[bot, c0], w[bot, c1])):
                    sums[k, top, c0] = t.astype(BF16)
            return carry
        lax.fori_loop(0, kh // step, body, 0)

    def rhs(w, sums, k, kh, nh, j, n):
        if k == 1:
            return w[:kh, pl.ds(j, n)]
        if k == 4:
            return w[kh:, pl.ds(nh + j, n)]
        return sums[SUMS.index(k), :, pl.ds(j, n)]

    def ffn_unit(i, l):
        for j in range(0, FH, 128):
            c0, c1 = pl.ds(j, 128), pl.ds(FH + j, 128)
            hs = []
            for c, cs in zip(_seven(lambda k: _dot(get_xt(k), rhs(w1, s1, k, DHF, FH, j, 128))),
                             (c0, c1, c0, c1)):
                hh = c + bb1[0:1, cs]
                rr = jnp.where(hh > 0, hh, 0.0)
                hs.append(rr * rr)
            for k, t in enumerate(_lhs7(*hs)):
                h[pl.ds(k * WH, WH), c0] = _pk(t)
        layernorm(xb, i + 1)
        for j in range(0, DHF, 256):
            ys = _seven(lambda k: _dot(_bf(h[pl.ds(k * WH, WH), :]), rhs(w2, s2, k, FH, DHF, j, 256)))
            for y, r, c in zip(ys, (0, 0, RH, RH), (j, DHF + j, j, DHF + j)):
                rows, cs = _rows(i * R + r, RH), pl.ds(c, 256)
                x2 = xb[rows, cs] + (y + bb2[0:1, cs])
                xa[rows, cs] = x2
                ostage[rows, cs] = x2.astype(BF16)

            @pl.when(l == LAYERS - 1)
            def _():
                for c in range(j // 128, j // 128 + 2):
                    cp_o(i, c).start()
                    cp_o(i, OC // 2 + c).start()

    cp_x(0).wait()
    for g in range(1, NG):
        for c in cp_q[g]:
            c.start()
    layernorm_first()
    first_unit()

    def layer(l, carry):
        def attn_step(i, c):
            @pl.when(jnp.logical_and(l == 0, i + 1 < NB))
            def _():
                cp_x(i + 1).wait()

            @pl.when(i == 1)
            def _():
                cp_ba.start()

            @pl.when(i == NB - 1)
            def _():
                cp_ba.wait()

            attn_unit(i, l)
            return c

        lax.fori_loop(jnp.where(l == 0, 1, 0), NB, attn_step, 0)

        @pl.when(l == 0)
        def _():
            cp_w1.wait()
            cp_w2.wait()
            prepare(w1, s1, DHF, FH, 16)
            prepare(w2, s2, FH, DHF, 32)

        def ffn_step(i, c):
            @pl.when(i == 1)
            def _():
                cp_ab.start()

            @pl.when(i == NB - 1)
            def _():
                cp_ab.wait()

            ffn_unit(i, l)
            return c

        lax.fori_loop(0, NB, ffn_step, 0)
        return carry

    lax.fori_loop(0, LAYERS, layer, 0)
    for i in range(NB):
        for c in range(OC):
            cp_o(i, c).wait()


@jax.jit
def pallas_interleave_layers__sliding_local_dilated__dense_activation_squared_relu__prompt_kernel(
    A_x: jax.Array,
    A_wqkv: jax.Array,
    A_wo: jax.Array,
    B_x: jax.Array,
    B_w1: jax.Array,
    B_b1: jax.Array,
    B_w2: jax.Array,
    B_b2: jax.Array,
):
    del B_x
    hbm = pl.BlockSpec(memory_space=pl.ANY)
    out = pl.pallas_call(
        _kernel,
        out_shape=jax.ShapeDtypeStruct((S, D), BF16),
        grid=(1,),
        in_specs=[hbm] * 7,
        out_specs=hbm,
        scratch_shapes=[
            pltpu.VMEM((S, D), BF16),
            pltpu.VMEM((D, 3 * D), BF16),
            pltpu.VMEM((D, D), BF16),
            pltpu.VMEM((D // 2, 3 * D), U32),
            pltpu.VMEM((5 * DHF // 2, 3 * DHF), U32),
            pltpu.VMEM((D // 2, D), U32),
            pltpu.VMEM((D, F), BF16),
            pltpu.VMEM((F, D), BF16),
            pltpu.VMEM((5, DHF, FH), BF16),
            pltpu.VMEM((5, FH, DHF), BF16),
            pltpu.VMEM((8, F), F32),
            pltpu.VMEM((8, D), F32),
            pltpu.VMEM((S + R, D), F32),
            pltpu.VMEM((XT0 + 4 * WH, D), F32),
            pltpu.VMEM((3 * D, 128), U32),
            pltpu.VMEM((3 * D // 2, R), U32),
            pltpu.VMEM((D, 128), U32),
            pltpu.VMEM((D, 128), U32),
            pltpu.VMEM((RH + 4 * WH, D), U32),
            pltpu.VMEM((7 * WH, FH), U32),
            pltpu.VMEM((S, D), BF16),
            pltpu.VMEM((F,), BF16),
            pltpu.VMEM((D,), BF16),
            pltpu.SemaphoreType.DMA((NB,)),
            pltpu.SemaphoreType.DMA((3 * NG,)),
            pltpu.SemaphoreType.DMA((6,)),
            pltpu.SemaphoreType.DMA((NB, OC)),
            pltpu.SemaphoreType.DMA((2,)),
            pltpu.SemaphoreType.REGULAR,
        ],
        compiler_params=pltpu.CompilerParams(vmem_limit_bytes=120 * 1024 * 1024),
    )(A_x.reshape(S, D), A_wqkv, A_wo, B_w1, B_b1, B_w2, B_b2)
    return out.reshape(1, S, D)
```
